```python
import jax
import jax.numpy as jnp

def _softmax(x, axis=-1):
    return jax.nn.softmax(x, axis=axis)

def _gelu(x):
    return jax.nn.gelu(x, approximate=True)

def _silu(x):
    return jax.nn.silu(x)

def _sigmoid(x):
    return jax.nn.sigmoid(x)

def _layernorm(x, axis=-1, eps=1e-05):
    m = jnp.mean(x, axis=axis, keepdims=True)
    v = jnp.var(x, axis=axis, keepdims=True)
    return (x - m) / jnp.sqrt(v + eps)

def _scatter_add(tgt, idx, src, axis=0):
    return tgt.at[idx].add(src)

def _segment_sum(src, seg, n):
    return jax.ops.segment_sum(src, seg, n)

class _Rng:

    def __init__(self, key):
        self._k = key

    def _next(self):
        self._k, sub = jax.random.split(self._k)
        return sub

    def normal(self, shape):
        return jax.random.normal(self._next(), shape, dtype=jnp.bfloat16)

    def randint(self, lo, hi, shape):
        return jax.random.randint(self._next(), shape, lo, hi, dtype=jnp.int32)

    def uniform(self, shape, lo=0.0, hi=1.0):
        return jax.random.uniform(self._next(), shape, jnp.bfloat16, lo, hi)

    def permutation(self, n):
        return jax.random.permutation(self._next(), n)
kernel_name = 'recurrent_scan__memory_aug_recurrent_mem_tr__mixer_s_mlp__prompt'

def setup_inputs():
    _rng = _Rng(jax.random.key(int.from_bytes(__import__("os").urandom(4), "little")))
    _w = lambda a: (lambda t: t.astype(jnp.bfloat16) if jnp.issubdtype(t.dtype, jnp.floating) else t)(jnp.asarray(a))

    def _A_setup():
        B, S, Dm = (1, 2048, 1024)
        H, Dh = (32, 128)
        M, seg = (8, 32)
        seg = min(seg, S)
        S = S // seg * seg
        return {'x': _w((lambda *s: _rng.normal(s) * 0.05)(B, S, Dm)), 'mem0': _w((lambda *s: _rng.normal(s) * 0.05)(B, M, Dm)), 'Wq': _w((lambda *s: _rng.normal(s) * 0.05)(Dm, H, Dh) * Dm ** (-0.5)), 'Wk': _w((lambda *s: _rng.normal(s) * 0.05)(Dm, H, Dh) * Dm ** (-0.5)), 'Wv': _w((lambda *s: _rng.normal(s) * 0.05)(Dm, H, Dh) * Dm ** (-0.5)), 'Wo': _w((lambda *s: _rng.normal(s) * 0.05)(H, Dh, Dm) * (H * Dh) ** (-0.5)), 'seg_len': seg}
    _A_in = _A_setup()

    def _B_setup():
        B, S, D, F = (1, 2048, 1024, 3584)
        return {'x': _w((lambda *s: _rng.normal(s) * 0.05)(B, S, D)), 'w1': _w((lambda *s: _rng.normal(s) * 0.05)(D, D) * D ** (-0.5)), 'w2': _w((lambda *s: _rng.normal(s) * 0.05)(D, D) * D ** (-0.5)), 'w3': _w((lambda *s: _rng.normal(s) * 0.05)(D, F) * D ** (-0.5)), 'w4': _w((lambda *s: _rng.normal(s) * 0.05)(F, D) * F ** (-0.5))}
    _B_in = _B_setup()
    return {'A_x': _A_in['x'], 'A_mem0': _A_in['mem0'], 'A_Wq': _A_in['Wq'], 'A_Wk': _A_in['Wk'], 'A_Wv': _A_in['Wv'], 'A_Wo': _A_in['Wo'], 'A_seg_len': _A_in['seg_len'], 'B_x': _B_in['x'], 'B_w1': _B_in['w1'], 'B_w2': _B_in['w2'], 'B_w3': _B_in['w3'], 'B_w4': _B_in['w4']}

def reference(A_x, A_mem0, A_Wq, A_Wk, A_Wv, A_Wo, A_seg_len, B_x, B_w1, B_w2, B_w3, B_w4):

    def _A_ref(x, mem0, Wq, Wk, Wv, Wo, seg_len):
        B, S, Dm = x.shape
        H, Dh = (Wq.shape[1], Wq.shape[2])
        M = mem0.shape[1]
        scale = Dh ** (-0.5)
        n_seg = S // seg_len
        L = M + seg_len
        idx = jnp.arange(L)
        mask = (idx[:, None] < M) | (idx[:, None] >= idx[None, :])
        mem = mem0
        outs = []
        for s in range(n_seg):
            xs = x[:, s * seg_len:(s + 1) * seg_len, :].copy()
            h = jnp.concatenate([mem, xs], axis=1)
            q = jnp.einsum('btd,dhe->bhte', h, Wq)
            k = jnp.einsum('btd,dhe->bhte', h, Wk)
            v = jnp.einsum('btd,dhe->bhte', h, Wv)
            scores = jnp.einsum('bhqe,bhke->bhqk', q, k) * scale
            scores = jnp.where(mask[None, None], scores, -1000000000.0)
            p = _softmax(scores, axis=-1)
            o = jnp.einsum('bhqk,bhke->bhqe', p, v)
            o = jnp.einsum('bhte,hed->btd', o, Wo)
            mem = o[:, :M, :].copy()
            outs.append(o[:, M:, :])
        return jnp.concatenate(outs, axis=1)

    def _B_ref(x, w1, w2, w3, w4):
        B, S, D = x.shape
        h = _gelu(_layernorm(x, axis=-1) @ w1)
        c = D // 4
        g0 = jnp.pad(h[:, :, 0 * c:1 * c], ((0, 0), (1, 0), (0, 0)))[:, :S, :]
        g1 = jnp.pad(h[:, :, 1 * c:2 * c], ((0, 0), (0, 1), (0, 0)))[:, 1:, :]
        g2 = jnp.pad(h[:, :, 2 * c:3 * c], ((0, 0), (2, 0), (0, 0)))[:, :S, :]
        g3 = jnp.pad(h[:, :, 3 * c:], ((0, 0), (0, 2), (0, 0)))[:, 2:, :]
        hs = jnp.concatenate([g0, g1, g2, g3], axis=-1) @ w2
        x1 = x + hs
        h2 = _gelu(_layernorm(x1, axis=-1) @ w3) @ w4
        return x1 + h2
    x = A_x
    xn = _layernorm(x, axis=-1)
    s = _A_ref(xn, A_mem0, A_Wq, A_Wk, A_Wv, A_Wo, A_seg_len)
    g = _silu(_B_ref(xn, B_w1, B_w2, B_w3, B_w4))
    return x + s * g
```

```python
import functools

import jax
import jax.numpy as jnp
from jax.experimental import pallas as pl
from jax.experimental.pallas import tpu as pltpu

_EPS = 1e-05
_LANES = 128
_PAD = 8
_TB = 256
_F32 = jnp.float32


def _layernorm(x):
    m = jnp.mean(x, axis=-1, keepdims=True)
    d = x - m
    v = jnp.mean(d * d, axis=-1, keepdims=True)
    return d * jax.lax.rsqrt(v + _EPS)


def _gelu(x):
    return jax.nn.gelu(x, approximate=True)


def _dot(a, b):
    return jnp.dot(a, b, preferred_element_type=_F32)


def _kernel(x_hbm, mem0_ref, wq_hbm, wk_hbm, wv_hbm, wo_hbm, w1_hbm, w2_hbm, w3_hbm, w4_hbm,
            out_hbm,
            x_v, xn_v, hb_v, gate_v, wqkv_v, wo_v, w1_v, w2_v, w3_v, w4_v, stage_v, h_v, o_v,
            sem_x, sem_w, sem_wo, sem_st, sem_out,
            *, seg, n_heads):
    S, D = x_v.shape
    M = mem0_ref.shape[0]
    L = M + seg
    H = n_heads
    n_blk = S // _TB
    n_seg = S // seg
    n_col = D // _LANES
    db = D // n_blk
    c = D // 4
    scale = _LANES ** (-0.5)

    def x_copy(i):
        rows = pl.ds(pl.multiple_of(i * _TB, _TB), _TB)
        return pltpu.make_async_copy(x_hbm.at[rows], x_v.at[rows], sem_x.at[i])

    def w_copies():
        pairs = ((w1_hbm, w1_v), (w2_hbm, w2_v), (w3_hbm, w3_v), (w4_hbm, w4_v))
        return [pltpu.make_async_copy(s, d, sem_w.at[j]) for j, (s, d) in enumerate(pairs)]

    def wo_copy(n):
        return pltpu.make_async_copy(wo_hbm.at[:, pl.ds(n * _LANES, _LANES)], wo_v.at[n],
                                     sem_wo.at[n])

    def stage_copy(i, j):
        src = (wq_hbm, wk_hbm, wv_hbm)[j]
        rows = pl.ds(pl.multiple_of(i * (db * H), db * H), db * H)
        slot = (i % 2) * 3 + j
        return pltpu.make_async_copy(src.at[rows], stage_v.at[slot], sem_st.at[slot])

    def out_copy(s):
        rows = pl.ds(pl.multiple_of(s * seg, seg), seg)
        return pltpu.make_async_copy(x_v.at[rows], out_hbm.at[rows], sem_out.at[0])

    wc = w_copies()
    x_copy(0).start()
    wc[0].start()
    for i in range(1, n_blk):
        x_copy(i).start()
    for cp in wc[1:]:
        cp.start()
    for j in range(3):
        stage_copy(0, j).start()

    hb_v[0:_PAD, :] = jnp.zeros((_PAD, D), _F32)
    hb_v[_PAD + S:, :] = jnp.zeros((_PAD, D), _F32)

    wc[0].wait()

    def b0(i, carry):
        r0 = pl.multiple_of(i * _TB, _TB)
        x_copy(i).wait()
        xn = _layernorm(x_v[pl.ds(r0, _TB), :].astype(_F32))
        xn_v[pl.ds(r0, _TB), :] = xn
        hb_v[pl.ds(r0 + _PAD, _TB), :] = _gelu(_dot(_layernorm(xn), w1_v[...]))
        return carry

    jax.lax.fori_loop(0, n_blk, b0, 0)

    for n in range(n_col):
        wo_copy(n).start()
    for cp in wc[1:]:
        cp.wait()
    stage_u = stage_v.bitcast(jnp.uint32)

    def b1(i, carry):
        r0 = pl.multiple_of(i * _TB, _TB)

        @pl.when(i + 1 < n_blk)
        def _():
            for j in range(3):
                stage_copy(i + 1, j).start()

        for j in range(3):
            stage_copy(i, j).wait()

        j0 = pl.multiple_of(i * (db // 2), db // 2)
        for j in range(3):
            w = stage_u[(i % 2) * 3 + j].reshape(db // 2, H, _LANES)
            a, b = w[:, :H // 2, :], w[:, H // 2:, :]
            even = jnp.transpose((a & jnp.uint32(0xFFFF)) | (b << 16), (1, 0, 2))
            odd = jnp.transpose((a >> 16) | (b & jnp.uint32(0xFFFF0000)), (1, 0, 2))
            for hp in range(H // 2):
                wqkv_v[(2 * hp) * 3 + j, pl.ds(j0, db // 2), :] = even[hp]
                wqkv_v[(2 * hp + 1) * 3 + j, pl.ds(j0, db // 2), :] = odd[hp]

        parts = []
        for q, shift in enumerate((-1, 1, -2, 2)):
            win = hb_v[pl.ds(r0, _TB + 2 * _PAD), q * c:(q + 1) * c]
            parts.append(win[_PAD + shift:_PAD + shift + _TB])
        x1 = xn_v[pl.ds(r0, _TB), :] + _dot(jnp.concatenate(parts, axis=1), w2_v[...])
        u = _gelu(_dot(_layernorm(x1).astype(jnp.bfloat16), w3_v[...]))
        y = x1 + _dot(u.astype(jnp.bfloat16), w4_v[...])
        gate_v[pl.ds(r0, _TB), :] = y * jax.nn.sigmoid(y)
        return carry

    jax.lax.fori_loop(0, n_blk, b1, 0)

    for n in range(n_col):
        wo_copy(n).wait()
    wo_u = wo_v.bitcast(jnp.uint32)
    h_v[0:M, :] = mem0_ref[...].astype(_F32)

    def proj(h, j):
        return _dot(h_v[...], pltpu.bitcast(wqkv_v[h * 3 + j], jnp.bfloat16))

    def step(s, carry):
        r0 = pl.multiple_of(s * seg, seg)
        h_v[M:L, :] = xn_v[pl.ds(r0, seg), :]
        qi = jax.lax.broadcasted_iota(jnp.int32, (L, L), 0)
        ki = jax.lax.broadcasted_iota(jnp.int32, (L, L), 1)
        mask = (qi < M) | (qi >= ki)

        qkv, prob = {}, {}
        for t in range(H + 2):
            if t < H:
                qkv[t] = (proj(t, 0), proj(t, 1), proj(t, 2))
            if 0 <= t - 1 < H:
                q, k, _ = qkv[t - 1]
                sc = jax.lax.dot_general(q, k, (((1,), (1,)), ((), ())),
                                         preferred_element_type=_F32)
                sc = jnp.where(mask, sc * scale, -1000000000.0)
                p = jnp.exp(sc - jnp.max(sc, axis=-1, keepdims=True))
                prob[t - 1] = p / jnp.sum(p, axis=-1, keepdims=True)
            if 0 <= t - 2 < H:
                hd = t - 2
                o_v[:, hd * _LANES:(hd + 1) * _LANES] = _dot(prob.pop(hd), qkv.pop(hd)[2])

        for n in range(n_col):
            cols = slice(n * _LANES, (n + 1) * _LANES)
            o = _dot(o_v[...], pltpu.bitcast(wo_u[n], jnp.bfloat16))
            h_v[0:M, cols] = o[0:M]
            res = (x_v[pl.ds(r0, seg), cols].astype(_F32)
                   + o[M:L] * gate_v[pl.ds(r0, seg), cols])
            x_v[pl.ds(r0, seg), cols] = res.astype(x_v.dtype)
        out_copy(s).start()
        return carry

    jax.lax.fori_loop(0, n_seg, step, 0)
    pltpu.make_async_copy(x_v, out_hbm, sem_out.at[0]).wait()


@functools.partial(jax.jit, static_argnames=("A_seg_len",))
def pallas_recurrent_scan__memory_aug_recurrent_mem_tr__mixer_s_mlp__prompt_kernel(
    A_x, A_mem0, A_Wq, A_Wk, A_Wv, A_Wo, A_seg_len, B_x, B_w1, B_w2, B_w3, B_w4,
):
    del B_x
    B, S, D = A_x.shape
    M = A_mem0.shape[1]
    _, H, Dh = A_Wq.shape
    F = B_w3.shape[1]
    seg = int(A_seg_len)
    assert B == 1 and Dh == _LANES and S % _TB == 0 and S % seg == 0
    n_blk = S // _TB
    n_col = D // _LANES
    bf16 = jnp.bfloat16

    any_spec = pl.BlockSpec(memory_space=pl.ANY)
    out = pl.pallas_call(
        functools.partial(_kernel, seg=seg, n_heads=H),
        out_shape=jax.ShapeDtypeStruct((S, D), A_x.dtype),
        in_specs=[any_spec, pl.BlockSpec(memory_space=pltpu.VMEM)] + [any_spec] * 8,
        out_specs=any_spec,
        scratch_shapes=[
            pltpu.VMEM((S, D), bf16),
            pltpu.VMEM((S, D), _F32),
            pltpu.VMEM((S + 2 * _PAD, D), _F32),
            pltpu.VMEM((S, D), _F32),
            pltpu.VMEM((3 * H, D // 2, Dh), jnp.uint32),
            pltpu.VMEM((n_col, H * Dh, _LANES), bf16),
            pltpu.VMEM((D, D), bf16),
            pltpu.VMEM((D, D), bf16),
            pltpu.VMEM((D, F), bf16),
            pltpu.VMEM((F, D), bf16),
            pltpu.VMEM((6, (D // n_blk) * H, Dh), bf16),
            pltpu.VMEM((M + seg, D), _F32),
            pltpu.VMEM((M + seg, H * Dh), _F32),
            pltpu.SemaphoreType.DMA((n_blk,)),
            pltpu.SemaphoreType.DMA((4,)),
            pltpu.SemaphoreType.DMA((n_col,)),
            pltpu.SemaphoreType.DMA((6,)),
            pltpu.SemaphoreType.DMA((1,)),
        ],
        compiler_params=pltpu.CompilerParams(vmem_limit_bytes=120 * 1024 * 1024),
    )(
        A_x.reshape(S, D), A_mem0.reshape(M, D),
        A_Wq.reshape(D * H, Dh), A_Wk.reshape(D * H, Dh), A_Wv.reshape(D * H, Dh),
        A_Wo.reshape(H * Dh, D), B_w1, B_w2, B_w3, B_w4,
    )
    return out.reshape(B, S, D)
```

```python
import functools

import jax
import jax.numpy as jnp
from jax.experimental import pallas as pl
from jax.experimental.pallas import tpu as pltpu

_EPS = 1e-05
_LANES = 128
_PAD = 8
_TB = 256
_F32 = jnp.float32


def _layernorm(x):
    m = jnp.mean(x, axis=-1, keepdims=True)
    d = x - m
    v = jnp.mean(d * d, axis=-1, keepdims=True)
    return d * jax.lax.rsqrt(v + _EPS)


def _gelu(x):
    return jax.nn.gelu(x, approximate=True)


def _dot(a, b):
    return jnp.dot(a, b, preferred_element_type=_F32)


def _kernel(x_hbm, mem0_ref, wq_hbm, wk_hbm, wv_hbm, wo_hbm, w1_hbm, w2_hbm, w3_hbm, w4_hbm,
            out_hbm,
            x_v, xn_v, hb_v, gate_v, wqkv_v, wo_v, w1_v, w2_v, w3_v, w4_v, stage_v, h_v, o_v, acc_v,
            sem_x, sem_w, sem_wo, sem_st, sem_out,
            *, seg, n_heads):
    S, D = x_v.shape
    M = mem0_ref.shape[0]
    L = M + seg
    H = n_heads
    n_blk = S // _TB
    n_seg = S // seg
    n_col = D // _LANES
    db = D // n_blk
    c = D // 4
    scale = _LANES ** (-0.5)

    def x_copy(i):
        rows = pl.ds(pl.multiple_of(i * _TB, _TB), _TB)
        return pltpu.make_async_copy(x_hbm.at[rows], x_v.at[rows], sem_x.at[i])

    def w_copies():
        pairs = ((w1_hbm, w1_v), (w2_hbm, w2_v), (w3_hbm, w3_v), (w4_hbm, w4_v))
        return [pltpu.make_async_copy(s, d, sem_w.at[j]) for j, (s, d) in enumerate(pairs)]

    def wo_copy(n):
        return pltpu.make_async_copy(wo_hbm.at[:, pl.ds(n * _LANES, _LANES)], wo_v.at[n],
                                     sem_wo.at[n])

    def stage_copy(i, j):
        src = (wq_hbm, wk_hbm, wv_hbm)[j]
        rows = pl.ds(pl.multiple_of(i * (db * H), db * H), db * H)
        slot = (i % 2) * 3 + j
        return pltpu.make_async_copy(src.at[rows], stage_v.at[slot], sem_st.at[slot])

    def out_copy(s):
        rows = pl.ds(pl.multiple_of(s * seg, seg), seg)
        return pltpu.make_async_copy(x_v.at[rows], out_hbm.at[rows], sem_out.at[0])

    wc = w_copies()
    x_copy(0).start()
    wc[0].start()
    for i in range(1, n_blk):
        x_copy(i).start()
    for cp in wc[1:]:
        cp.start()
    for j in range(3):
        stage_copy(0, j).start()

    hb_v[0:_PAD, :] = jnp.zeros((_PAD, D), _F32)
    hb_v[_PAD + S:, :] = jnp.zeros((_PAD, D), _F32)

    def norms(i):
        r0 = pl.multiple_of(i * _TB, _TB)
        xn = _layernorm(x_v[pl.ds(r0, _TB), :].astype(_F32))
        xn_v[pl.ds(r0, _TB), :] = xn
        gate_v[pl.ds(r0, _TB), :] = _layernorm(xn)

    x_copy(0).wait()
    norms(0)
    with jax.named_scope('wait_w1'):
        wc[0].wait()

    def b0(i, carry):
        nxt = jnp.minimum(i + 1, n_blk - 1)

        @pl.when(i + 1 < n_blk)
        def _():
            x_copy(i + 1).wait()

        r0 = pl.multiple_of(i * _TB, _TB)
        hb_v[pl.ds(r0 + _PAD, _TB), :] = _gelu(_dot(gate_v[pl.ds(r0, _TB), :], w1_v[...]))
        norms(nxt)
        return carry

    with jax.named_scope('B0'):
        jax.lax.fori_loop(0, n_blk, b0, 0)

    for n in range(n_col):
        wo_copy(n).start()
    for cp in wc[1:]:
        cp.wait()
    stage_u = stage_v.bitcast(jnp.uint32)

    def b1(i, carry):
        @pl.when(i + 1 < n_blk)
        def _():
            for j in range(3):
                stage_copy(i + 1, j).start()

        for j in range(3):
            stage_copy(i, j).wait()

        def relayout(j):
            slot = (i % 2) * 3 + j
            for g in range(db // 16):
                j0 = pl.multiple_of(i * (db // 2) + g * 8, 8)
                w = stage_u[slot, g * 8 * H:(g + 1) * 8 * H, :].reshape(8, H, _LANES)
                for t in range(H // 16):
                    a = w[:, 8 * t:8 * t + 8, :]
                    b = w[:, H // 2 + 8 * t:H // 2 + 8 * t + 8, :]
                    even = jnp.transpose((a & jnp.uint32(0xFFFF)) | (b << 16), (1, 0, 2))
                    odd = jnp.transpose((a >> 16) | (b & jnp.uint32(0xFFFF0000)), (1, 0, 2))
                    for r in range(8):
                        hp = 8 * t + r
                        wqkv_v[(2 * hp) * 3 + j, pl.ds(j0, 8), :] = even[r]
                        wqkv_v[(2 * hp + 1) * 3 + j, pl.ds(j0, 8), :] = odd[r]

        hb = _TB // 2

        def mix(r0):
            parts = []
            for q, shift in enumerate((-1, 1, -2, 2)):
                win = hb_v[pl.ds(r0, hb + 2 * _PAD), q * c:(q + 1) * c]
                parts.append(win[_PAD + shift:_PAD + shift + hb])
            return xn_v[pl.ds(r0, hb), :] + _dot(jnp.concatenate(parts, axis=1), w2_v[...])

        def up(x1):
            return _gelu(_dot(_layernorm(x1).astype(jnp.bfloat16), w3_v[...])).astype(jnp.bfloat16)

        def down(r0, x1, u):
            y = x1 + _dot(u, w4_v[...])
            gate_v[pl.ds(r0, hb), :] = y * jax.nn.sigmoid(y)

        ra = pl.multiple_of(i * _TB, hb)
        rb = pl.multiple_of(i * _TB + hb, hb)
        xa = mix(ra)
        xb = mix(rb)
        ua = up(xa)
        relayout(0)
        ub = up(xb)
        relayout(1)
        down(ra, xa, ua)
        relayout(2)
        down(rb, xb, ub)
        return carry

    with jax.named_scope('B1'):
        jax.lax.fori_loop(0, n_blk, b1, 0)

    for n in range(n_col):
        wo_copy(n).wait()
    wo_u = wo_v.bitcast(jnp.uint32)
    h_v[0:M, :] = mem0_ref[...].astype(_F32)
    h_early = H - H // 4

    def proj(h, j):
        return _dot(h_v[...], pltpu.bitcast(wqkv_v[h * 3 + j], jnp.bfloat16))

    def out_proj(n, h0, h1):
        w = wo_u[n, h0 * (_LANES // 2):h1 * (_LANES // 2), :]
        return _dot(o_v[:, h0 * _LANES:h1 * _LANES], pltpu.bitcast(w, jnp.bfloat16))

    def step(s, carry):
        r0 = pl.multiple_of(s * seg, seg)
        h_v[M:L, :] = xn_v[pl.ds(r0, seg), :]
        qi = jax.lax.broadcasted_iota(jnp.int32, (L, L), 0)
        ki = jax.lax.broadcasted_iota(jnp.int32, (L, L), 1)
        mask = (qi < M) | (qi >= ki)
        qkv, prob = {}, {}

        def scores(h):
            q, k, _ = qkv[h]
            sc = jax.lax.dot_general(q, k, (((1,), (1,)), ((), ())),
                                     preferred_element_type=_F32)
            sc = jnp.where(mask, sc * scale, -1000000000.0)
            p = jnp.exp(sc - jnp.max(sc, axis=-1, keepdims=True))
            prob[h] = p / jnp.sum(p, axis=-1, keepdims=True)

        def values(h):
            o_v[:, h * _LANES:(h + 1) * _LANES] = _dot(prob.pop(h), qkv.pop(h)[2])

        for t in range(H):
            qkv[t] = (proj(t, 0), proj(t, 1), proj(t, 2))
            if t >= 1:
                scores(t - 1)
            if t >= 2:
                values(t - 2)

        for n in range(n_col):
            acc_v[:, n * _LANES:(n + 1) * _LANES] = out_proj(n, 0, h_early)
            if n == 0:
                scores(H - 1)
            if n == 1:
                values(H - 2)
            if n == 3:
                values(H - 1)

        for n in range(n_col):
            cols = slice(n * _LANES, (n + 1) * _LANES)
            o = acc_v[:, cols] + out_proj(n, h_early, H)
            h_v[0:M, cols] = o[0:M]
            res = (x_v[pl.ds(r0, seg), cols].astype(_F32)
                   + o[M:L] * gate_v[pl.ds(r0, seg), cols])
            x_v[pl.ds(r0, seg), cols] = res.astype(x_v.dtype)
        out_copy(s).start()
        return carry

    with jax.named_scope('A'):
        jax.lax.fori_loop(0, n_seg, step, 0)
    pltpu.make_async_copy(x_v, out_hbm, sem_out.at[0]).wait()


@functools.partial(jax.jit, static_argnames=("A_seg_len",))
def pallas_recurrent_scan__memory_aug_recurrent_mem_tr__mixer_s_mlp__prompt_kernel(
    A_x, A_mem0, A_Wq, A_Wk, A_Wv, A_Wo, A_seg_len, B_x, B_w1, B_w2, B_w3, B_w4,
):
    del B_x
    B, S, D = A_x.shape
    M = A_mem0.shape[1]
    _, H, Dh = A_Wq.shape
    F = B_w3.shape[1]
    seg = int(A_seg_len)
    assert B == 1 and Dh == _LANES and S % _TB == 0 and S % seg == 0
    n_blk = S // _TB
    n_col = D // _LANES
    bf16 = jnp.bfloat16

    any_spec = pl.BlockSpec(memory_space=pl.ANY)
    out = pl.pallas_call(
        functools.partial(_kernel, seg=seg, n_heads=H),
        out_shape=jax.ShapeDtypeStruct((S, D), A_x.dtype),
        in_specs=[any_spec, pl.BlockSpec(memory_space=pltpu.VMEM)] + [any_spec] * 8,
        out_specs=any_spec,
        scratch_shapes=[
            pltpu.VMEM((S, D), bf16),
            pltpu.VMEM((S, D), _F32),
            pltpu.VMEM((S + 2 * _PAD, D), _F32),
            pltpu.VMEM((S, D), _F32),
            pltpu.VMEM((3 * H, D // 2, Dh), jnp.uint32),
            pltpu.VMEM((n_col, H * Dh, _LANES), bf16),
            pltpu.VMEM((D, D), bf16),
            pltpu.VMEM((D, D), bf16),
            pltpu.VMEM((D, F), bf16),
            pltpu.VMEM((F, D), bf16),
            pltpu.VMEM((6, (D // n_blk) * H, Dh), bf16),
            pltpu.VMEM((M + seg, D), _F32),
            pltpu.VMEM((M + seg, H * Dh), _F32),
            pltpu.VMEM((M + seg, D), _F32),
            pltpu.SemaphoreType.DMA((n_blk,)),
            pltpu.SemaphoreType.DMA((4,)),
            pltpu.SemaphoreType.DMA((n_col,)),
            pltpu.SemaphoreType.DMA((6,)),
            pltpu.SemaphoreType.DMA((1,)),
        ],
        compiler_params=pltpu.CompilerParams(vmem_limit_bytes=120 * 1024 * 1024),
    )(
        A_x.reshape(S, D), A_mem0.reshape(M, D),
        A_Wq.reshape(D * H, Dh), A_Wk.reshape(D * H, Dh), A_Wv.reshape(D * H, Dh),
        A_Wo.reshape(H * Dh, D), B_w1, B_w2, B_w3, B_w4,
    )
    return out.reshape(B, S, D)
```

```python
import functools

import jax
import jax.numpy as jnp
from jax.experimental import pallas as pl
from jax.experimental.pallas import tpu as pltpu

_EPS = 1e-05
_LANES = 128
_PAD = 8
_TB = 256
_TR = _TB
_TQ = 256
_LAG_S = 1
_LAG_V = 3
_F32 = jnp.float32
_BF16 = jnp.bfloat16
_U32 = jnp.uint32
UNROLL = 2
P_COLS = 6
P_ROWS = 16
R_COLS = 6
L3_LO = 0
L3_HI = 4
L3_ROWS = 32
N_UP = 96


def _layernorm(x):
    m = jnp.mean(x, axis=-1, keepdims=True)
    d = x - m
    v = jnp.mean(d * d, axis=-1, keepdims=True)
    return d * jax.lax.rsqrt(v + _EPS)


def _gelu(x):
    return jax.nn.gelu(x, approximate=True)


def _dot(a, b):
    return jnp.dot(a, b, preferred_element_type=_F32)


def _matmul(a, w_v):
    w = w_v.bitcast(_U32)
    lhs = a if callable(a) else lambda: a
    return jnp.concatenate(
        [_dot(lhs(), pltpu.bitcast(w[n], _BF16)) for n in range(w_v.shape[0])], axis=1)


def _anchors(val, count, zero):
    cols = val.shape[1] // _LANES
    per = -(-count // cols)
    out = []
    for p in range(count):
        n, r = divmod(p * cols * per // count, per)
        r0 = r * (val.shape[0] // per) // 8 * 8
        out.append(pltpu.bitcast(val[r0:r0 + 8, n * _LANES:(n + 1) * _LANES], _U32) & zero)
    return out


def _kernel(x_hbm, mem0_ref, wq_hbm, wk_hbm, wv_hbm, wo_hbm, w1_hbm, w2_hbm, w3_hbm, w4_hbm,
            out_hbm,
            x_v, xn_v, hb_v, x1_v, la_v, lb_v, wqkv_v, wo_v, w1_v, w2_v, w3_v, w4_v, stage_v,
            h_v, o_v, acc_v,
            sem_x, sem_w, sem_st, sem_out,
            *, seg, n_heads):
    S, D = x_v.shape
    M = mem0_ref.shape[0]
    L = M + seg
    H = n_heads
    n_blk = S // _TB
    n_mlp = S // _TR
    n_seg = S // seg
    n_col = D // _LANES
    db = D // n_mlp
    c = D // 4
    scale = _LANES ** (-0.5)

    def x_copy(i):
        rows = pl.ds(pl.multiple_of(i * _TB, _TB), _TB)
        return pltpu.make_async_copy(x_hbm.at[rows], x_v.at[rows], sem_x.at[i])

    w_pairs = ((w1_hbm, w1_v), (w2_hbm, w2_v), (w3_hbm, w3_v), (w4_hbm, w4_v), (wo_hbm, wo_v))

    def w_start(j, part=0, parts=1):
        src, dst = w_pairs[j]
        per = dst.shape[0] // parts
        for n in range(part * per, (part + 1) * per):
            pltpu.make_async_copy(src.at[:, pl.ds(n * _LANES, _LANES)], dst.at[n],
                                  sem_w.at[j]).start()

    def w_wait(j):
        dst = w_pairs[j][1]
        pltpu.make_async_copy(dst, dst, sem_w.at[j]).wait()

    def stage_copy(i, j):
        src = (wq_hbm, wk_hbm, wv_hbm)[j]
        rows = pl.ds(pl.multiple_of(i * (db * H), db * H), db * H)
        slot = (i % 2) * 3 + j
        return pltpu.make_async_copy(src.at[rows], stage_v.at[slot], sem_st.at[slot])

    def stage_start(i):
        for j in range(3):
            stage_copy(i, j).start()

    def out_copy(s):
        rows = pl.ds(pl.multiple_of(s * seg, seg), seg)
        return pltpu.make_async_copy(x_v.at[rows], out_hbm.at[rows], sem_out.at[0])

    def paced(i, steps, jobs):
        per = -(-len(jobs) // steps)
        for k in range(steps):
            mine = jobs[k * per:(k + 1) * per]
            if mine:
                @pl.when(i == k)
                def _(mine=mine):
                    for job in mine:
                        job()

    part = functools.partial
    jobs_p = [part(w_start, 1), part(w_start, 2, 0, 4), part(w_start, 2, 1, 4),
              part(w_start, 2, 2, 4)]
    jobs_q = ([part(w_start, 2, 3, 4)] + [part(w_start, 3, k, 4) for k in range(4)]
              + [part(stage_start, 0)] + [part(w_start, 4, k, 2) for k in range(2)])

    x_copy(0).start()
    w_start(0)
    x_copy(1).start()
    x_copy(2).start()
    hb_v[0:_PAD, :] = jnp.zeros((_PAD, D), _F32)
    hb_v[_PAD + S:, :] = jnp.zeros((_PAD, D), _F32)

    def norms(dst_v, src0, dst0, rows, z=None):
        x = x_v[pl.ds(src0, rows), :]
        if z is not None:
            words = pltpu.bitcast(x, _U32) | jnp.tile(z, (rows // 16, n_col))
            x = pltpu.bitcast(words, _BF16)
        xn = _layernorm(x.astype(_F32))
        xn_v[pl.ds(src0, rows), :] = xn
        dst_v[pl.ds(dst0 // 2, rows // 2), :] = pltpu.bitcast(_layernorm(xn).astype(_BF16), _U32)

    x_copy(0).wait()
    norms(la_v, 0, 0, _TB)
    w_wait(0)

    def phase_p(i, carry):
        paced(i, n_blk // 2, jobs_p)
        for k in (3, 4):
            @pl.when(2 * i + k < n_blk)
            def _():
                x_copy(2 * i + k).start()

        x_copy(2 * i + 1).wait()

        @pl.when(2 * i + 2 < n_blk)
        def _():
            x_copy(2 * i + 2).wait()

        zero = pltpu.bitcast(hb_v[0:8, 0:_LANES], _U32)
        for k, (cur_v, nxt_v) in enumerate(((la_v, lb_v), (lb_v, la_v))):
            blk = 2 * i + k
            r0 = pl.multiple_of(blk * _TB, _TB)
            pre = _matmul(lambda: pltpu.bitcast(cur_v[...], _BF16), w1_v)
            hb_v[pl.ds(r0 + _PAD, _TB), :] = _gelu(pre)
            nxt = jnp.minimum(blk + 1, n_blk - 1) * _TB
            rows = P_ROWS
            for g, z in enumerate(_anchors(pre[:, :P_COLS * _LANES], _TB // rows, zero)):
                norms(nxt_v, pl.multiple_of(nxt + g * rows, rows), g * rows, rows, z)
        return carry

    jax.lax.fori_loop(0, n_blk // 2, phase_p, 0)

    w_wait(1)

    def phase_q(i, carry):
        paced(i, S // _TQ, jobs_q)
        r0 = pl.multiple_of(i * _TQ, _TQ)
        parts = []
        for q, shift in enumerate((-1, 1, -2, 2)):
            win = hb_v[pl.ds(r0, _TQ + 2 * _PAD), q * c:(q + 1) * c]
            parts.append(win[_PAD + shift:_PAD + shift + _TQ])
        x1_v[pl.ds(r0, _TQ), :] = (xn_v[pl.ds(r0, _TQ), :]
                                     + _matmul(jnp.concatenate(parts, axis=1), w2_v))
        return carry

    jax.lax.fori_loop(0, S // _TQ, phase_q, 0)

    def norm3(src0, dst0, rows, z=None):
        x1 = x1_v[pl.ds(src0, rows), :]
        if z is not None:
            x1 = pltpu.bitcast(pltpu.bitcast(x1, _U32) | jnp.tile(z, (rows // 8, n_col)), _F32)
        la_v[pl.ds(dst0 // 2, rows // 2), :] = pltpu.bitcast(
            _layernorm(x1).astype(_BF16), _U32)

    norm3(0, 0, _TR)
    w_wait(2)
    w_wait(3)
    stage_u = stage_v.bitcast(_U32)

    def phase_r(i, carry):
        @pl.when(i + 1 < n_mlp)
        def _():
            stage_start(i + 1)

        for j in range(3):
            stage_copy(i, j).wait()

        zero = pltpu.bitcast(hb_v[0:8, 0:_LANES], _U32)

        def relayout(j, g, t, par, z):
            keep, sh = z | _U32(0xFFFF0000 if par else 0xFFFF), z | _U32(16)
            j0 = pl.multiple_of(i * (db // 2) + g * 8, 8)
            w = stage_u[(i % 2) * 3 + j, g * 8 * H:(g + 1) * 8 * H, :].reshape(8, H, _LANES)
            a = w[:, 8 * t:8 * t + 8, :]
            b = w[:, H // 2 + 8 * t:H // 2 + 8 * t + 8, :]
            word = ((a >> sh) | (b & keep)) if par else ((a & keep) | (b << sh))
            word = jnp.transpose(word, (1, 0, 2))
            for r in range(8):
                wqkv_v[(2 * (8 * t + r) + par) * 3 + j, pl.ds(j0, 8), :] = word[r]

        pieces = [(j, g, t, par) for j in range(3) for g in range(db // 16)
                  for t in range(H // 16) for par in range(2)]

        r0 = pl.multiple_of(i * _TR, _TR)
        pre = _matmul(lambda: pltpu.bitcast(la_v[...], _BF16), w3_v)
        for z in _anchors(pre, N_UP, zero):
            relayout(*pieces.pop(), z)
        y = x1_v[pl.ds(r0, _TR), :] + _matmul(_gelu(pre).astype(_BF16), w4_v)
        for z in _anchors(y[:, :R_COLS * _LANES], len(pieces), zero):
            relayout(*pieces.pop(), z)
        nxt = jnp.minimum(i + 1, n_mlp - 1) * _TR
        rows = L3_ROWS
        for g, z in enumerate(_anchors(y[:, L3_LO * _LANES:L3_HI * _LANES], _TR // rows, zero)):
            norm3(pl.multiple_of(nxt + g * rows, rows), g * rows, rows, z)
        hb_v[pl.ds(r0 + _PAD, _TR), :] = y * jax.nn.sigmoid(y)
        return carry

    jax.lax.fori_loop(0, n_mlp, phase_r, 0)

    w_wait(4)
    wo_u = wo_v.bitcast(_U32)
    h_v[0:M, :] = mem0_ref[...].astype(_F32)
    h_early = H - H // 4

    def proj(h, j):
        return _dot(h_v[...], pltpu.bitcast(wqkv_v[h * 3 + j], _BF16))

    def out_proj(n, h0, h1):
        w = wo_u[n, h0 * (_LANES // 2):h1 * (_LANES // 2), :]
        return _dot(o_v[:, h0 * _LANES:h1 * _LANES], pltpu.bitcast(w, _BF16))

    def step(s, carry):
        r0 = pl.multiple_of(s * seg, seg)
        h_v[M:L, :] = xn_v[pl.ds(r0, seg), :]
        qi = jax.lax.broadcasted_iota(jnp.int32, (L, L), 0)
        ki = jax.lax.broadcasted_iota(jnp.int32, (L, L), 1)
        mask = (qi < M) | (qi >= ki)
        qkv, prob = {}, {}

        def scores(h):
            q, k, _ = qkv[h]
            sc = jax.lax.dot_general(q, k, (((1,), (1,)), ((), ())),
                                     preferred_element_type=_F32)
            sc = jnp.where(mask, sc * scale, -1000000000.0)
            p = jnp.exp(sc - jnp.max(sc, axis=-1, keepdims=True))
            prob[h] = p / jnp.sum(p, axis=-1, keepdims=True)

        def values(h):
            o_v[:, h * _LANES:(h + 1) * _LANES] = _dot(prob.pop(h), qkv.pop(h)[2])

        for t in range(H + n_col):
            if t < H:
                qkv[t] = (proj(t, 0), proj(t, 1), proj(t, 2))
            else:
                n = t - H
                acc_v[:, n * _LANES:(n + 1) * _LANES] = out_proj(n, 0, h_early)
            if 0 <= t - _LAG_S < H:
                scores(t - _LAG_S)
            if 0 <= t - _LAG_V < H:
                values(t - _LAG_V)

        for n in range(n_col):
            cols = slice(n * _LANES, (n + 1) * _LANES)
            o = acc_v[:, cols] + out_proj(n, h_early, H)
            h_v[0:M, cols] = o[0:M]
            res = (x_v[pl.ds(r0, seg), cols].astype(_F32)
                   + o[M:L] * hb_v[pl.ds(r0 + _PAD, seg), cols])
            x_v[pl.ds(r0, seg), cols] = res.astype(x_v.dtype)
        out_copy(s).start()
        return carry

    jax.lax.fori_loop(0, n_seg, step, 0, unroll=UNROLL)
    pltpu.make_async_copy(x_v, out_hbm, sem_out.at[0]).wait()


@functools.partial(jax.jit, static_argnames=("A_seg_len",))
def pallas_recurrent_scan__memory_aug_recurrent_mem_tr__mixer_s_mlp__prompt_kernel(
    A_x, A_mem0, A_Wq, A_Wk, A_Wv, A_Wo, A_seg_len, B_x, B_w1, B_w2, B_w3, B_w4,
):
    del B_x
    B, S, D = A_x.shape
    M = A_mem0.shape[1]
    _, H, Dh = A_Wq.shape
    F = B_w3.shape[1]
    seg = int(A_seg_len)
    assert B == 1 and Dh == _LANES and S % _TB == 0 and S % _TR == 0 and S % seg == 0
    n_col = D // _LANES

    any_spec = pl.BlockSpec(memory_space=pl.ANY)
    out = pl.pallas_call(
        functools.partial(_kernel, seg=seg, n_heads=H),
        out_shape=jax.ShapeDtypeStruct((S, D), A_x.dtype),
        in_specs=[any_spec, pl.BlockSpec(memory_space=pltpu.VMEM)] + [any_spec] * 8,
        out_specs=any_spec,
        scratch_shapes=[
            pltpu.VMEM((S, D), _BF16),
            pltpu.VMEM((S, D), _F32),
            pltpu.VMEM((S + 2 * _PAD, D), _F32),
            pltpu.VMEM((S, D), _F32),
            pltpu.VMEM((_TB // 2, D), _U32),
            pltpu.VMEM((_TB // 2, D), _U32),
            pltpu.VMEM((3 * H, D // 2, Dh), _U32),
            pltpu.VMEM((n_col, H * Dh, _LANES), _BF16),
            pltpu.VMEM((n_col, D, _LANES), _BF16),
            pltpu.VMEM((n_col, D, _LANES), _BF16),
            pltpu.VMEM((F // _LANES, D, _LANES), _BF16),
            pltpu.VMEM((n_col, F, _LANES), _BF16),
            pltpu.VMEM((6, (D // (S // _TR)) * H, Dh), _BF16),
            pltpu.VMEM((M + seg, D), _F32),
            pltpu.VMEM((M + seg, H * Dh), _F32),
            pltpu.VMEM((M + seg, D), _F32),
            pltpu.SemaphoreType.DMA((S // _TB,)),
            pltpu.SemaphoreType.DMA((5,)),
            pltpu.SemaphoreType.DMA((6,)),
            pltpu.SemaphoreType.DMA((1,)),
        ],
        compiler_params=pltpu.CompilerParams(vmem_limit_bytes=120 * 1024 * 1024),
    )(
        A_x.reshape(S, D), A_mem0.reshape(M, D),
        A_Wq.reshape(D * H, Dh), A_Wk.reshape(D * H, Dh), A_Wv.reshape(D * H, Dh),
        A_Wo.reshape(H * Dh, D), B_w1, B_w2, B_w3, B_w4,
    )
    return out.reshape(B, S, D)
```

```python
import functools

import jax
import jax.numpy as jnp
from jax.experimental import pallas as pl
from jax.experimental.pallas import tpu as pltpu

_EPS = 1e-05
_LANES = 128
_PAD = 8
_TB = 256
_LAG_S = 1
_LAG_V = 3
_F32 = jnp.float32
_BF16 = jnp.bfloat16
_U32 = jnp.uint32


def _layernorm(x):
    m = jnp.mean(x, axis=-1, keepdims=True)
    d = x - m
    v = jnp.mean(d * d, axis=-1, keepdims=True)
    return d * jax.lax.rsqrt(v + _EPS)


def _gelu(x):
    return jax.nn.gelu(x, approximate=True)


def _dot(a, b):
    return jnp.dot(a, b, preferred_element_type=_F32)


def _matmul(a, w_v):
    w = w_v.bitcast(_U32)
    return jnp.concatenate(
        [_dot(a, pltpu.bitcast(w[n], _BF16)) for n in range(w_v.shape[0])], axis=1)


def _anchors(val, count, zero):
    cols = val.shape[1] // _LANES
    per = -(-count // cols)
    out = []
    for p in range(count):
        n, r = divmod(p * cols * per // count, per)
        r0 = r * (val.shape[0] // per) // 8 * 8
        out.append(pltpu.bitcast(val[r0:r0 + 8, n * _LANES:(n + 1) * _LANES], _U32) & zero)
    return out


def _kernel(x_hbm, mem0_hbm, wq_hbm, wk_hbm, wv_hbm, wo_hbm, w1_hbm, w2_hbm, w3_hbm, w4_hbm,
            out_hbm,
            x_v, xn_v, hb_v, x1_v, la_v, lb_v, wqkv_v, wo_v, w1_v, w2_v, w3_v, w4_v, stage_v,
            h_v, o_v, acc_v, mem0_v,
            sem_x, sem_w, sem_st, sem_io,
            *, seg, n_heads):
    S, D = x_v.shape
    M = mem0_v.shape[0]
    L = M + seg
    H = n_heads
    n_blk = S // _TB
    n_seg = S // seg
    n_col = D // _LANES
    db = D // n_blk
    c = D // 4
    scale = _LANES ** (-0.5)

    def x_copy(i):
        rows = pl.ds(pl.multiple_of(i * _TB, _TB), _TB)
        return pltpu.make_async_copy(x_hbm.at[rows], x_v.at[rows], sem_x.at[i])

    w_pairs = ((w1_hbm, w1_v), (w2_hbm, w2_v), (w3_hbm, w3_v), (w4_hbm, w4_v), (wo_hbm, wo_v))

    def w_start(j, part=0, parts=1):
        src, dst = w_pairs[j]
        tiles = dst.shape[0]
        for n in range(part * tiles // parts, (part + 1) * tiles // parts):
            pltpu.make_async_copy(src.at[:, pl.ds(n * _LANES, _LANES)], dst.at[n],
                                  sem_w.at[j]).start()

    def w_wait(j):
        dst = w_pairs[j][1]
        pltpu.make_async_copy(dst, dst, sem_w.at[j]).wait()

    def stage_copy(i, j):
        src = (wq_hbm, wk_hbm, wv_hbm)[j]
        rows = pl.ds(pl.multiple_of(i * (db * H), db * H), db * H)
        slot = (i % 2) * 3 + j
        return pltpu.make_async_copy(src.at[rows], stage_v.at[slot], sem_st.at[slot])

    def stage_start(i):
        for j in range(3):
            stage_copy(i, j).start()

    def out_copy(s):
        rows = pl.ds(pl.multiple_of(s * seg, seg), seg)
        return pltpu.make_async_copy(x_v.at[rows], out_hbm.at[rows], sem_io.at[0])

    mem0_copy = pltpu.make_async_copy(mem0_hbm, mem0_v, sem_io.at[1])

    def paced(i, steps, jobs):
        per = -(-len(jobs) // steps)
        for k in range(steps):
            mine = jobs[k * per:(k + 1) * per]
            if mine:
                @pl.when(i == k)
                def _(mine=mine):
                    for job in mine:
                        job()

    part = functools.partial
    jobs_p = [part(w_start, 1)] + [part(w_start, 2, k, 4) for k in range(3)]
    jobs_q = ([part(w_start, 2, 3, 4)] + [part(w_start, 3, k, 4) for k in range(4)]
              + [part(stage_start, 0)] + [part(w_start, 4, k, 2) for k in range(2)])

    x_copy(0).start()
    w_start(0)
    x_copy(1).start()
    x_copy(2).start()
    hb_v[0:_PAD, :] = jnp.zeros((_PAD, D), _F32)
    hb_v[_PAD + S:, :] = jnp.zeros((_PAD, D), _F32)

    def norms(dst_v, src0, dst0, rows, z=None):
        x = x_v[pl.ds(src0, rows), :]
        if z is not None:
            words = pltpu.bitcast(x, _U32) | jnp.tile(z, (rows // 16, n_col))
            x = pltpu.bitcast(words, _BF16)
        xn = _layernorm(x.astype(_F32))
        xn_v[pl.ds(src0, rows), :] = xn
        dst_v[pl.ds(dst0 // 2, rows // 2), :] = pltpu.bitcast(_layernorm(xn).astype(_BF16), _U32)

    x_copy(0).wait()
    norms(la_v, 0, 0, _TB)
    mem0_copy.start()
    w_wait(0)

    def phase_p(i, carry):
        paced(i, n_blk // 2, jobs_p)
        for k in (3, 4):
            @pl.when(2 * i + k < n_blk)
            def _(k=k):
                x_copy(2 * i + k).start()

        x_copy(2 * i + 1).wait()

        @pl.when(2 * i + 2 < n_blk)
        def _():
            x_copy(2 * i + 2).wait()

        zero = pltpu.bitcast(hb_v[0:8, 0:_LANES], _U32)
        for k, (cur_v, nxt_v) in enumerate(((la_v, lb_v), (lb_v, la_v))):
            blk = 2 * i + k
            r0 = pl.multiple_of(blk * _TB, _TB)
            pre = _matmul(pltpu.bitcast(cur_v[...], _BF16), w1_v)
            hb_v[pl.ds(r0 + _PAD, _TB), :] = _gelu(pre)
            nxt = jnp.minimum(blk + 1, n_blk - 1) * _TB
            rows = 16
            for g, z in enumerate(_anchors(pre[:, :3 * D // 4], _TB // rows, zero)):
                norms(nxt_v, pl.multiple_of(nxt + g * rows, rows), g * rows, rows, z)
        return carry

    jax.lax.fori_loop(0, n_blk // 2, phase_p, 0)

    w_wait(1)

    def phase_q(i, carry):
        paced(i, n_blk, jobs_q)
        r0 = pl.multiple_of(i * _TB, _TB)
        parts = []
        for q, shift in enumerate((-1, 1, -2, 2)):
            win = hb_v[pl.ds(r0, _TB + 2 * _PAD), q * c:(q + 1) * c]
            parts.append(win[_PAD + shift:_PAD + shift + _TB])
        x1_v[pl.ds(r0, _TB), :] = (xn_v[pl.ds(r0, _TB), :]
                                   + _matmul(jnp.concatenate(parts, axis=1), w2_v))
        return carry

    jax.lax.fori_loop(0, n_blk, phase_q, 0)

    def norm3(src0, dst0, rows, z=None):
        x1 = x1_v[pl.ds(src0, rows), :]
        if z is not None:
            x1 = pltpu.bitcast(pltpu.bitcast(x1, _U32) | jnp.tile(z, (rows // 8, n_col)), _F32)
        la_v[pl.ds(dst0 // 2, rows // 2), :] = pltpu.bitcast(_layernorm(x1).astype(_BF16), _U32)

    norm3(0, 0, _TB)
    w_wait(2)
    w_wait(3)
    stage_u = stage_v.bitcast(_U32)

    def phase_r(i, carry):
        @pl.when(i + 1 < n_blk)
        def _():
            stage_start(i + 1)

        for j in range(3):
            stage_copy(i, j).wait()

        zero = pltpu.bitcast(hb_v[0:8, 0:_LANES], _U32)

        def relayout(j, g, t, odd, z):
            keep, sh = z | _U32(0xFFFF0000 if odd else 0xFFFF), z | _U32(16)
            j0 = pl.multiple_of(i * (db // 2) + g * 8, 8)
            w = stage_u[(i % 2) * 3 + j, g * 8 * H:(g + 1) * 8 * H, :].reshape(8, H, _LANES)
            a = w[:, 8 * t:8 * t + 8, :]
            b = w[:, H // 2 + 8 * t:H // 2 + 8 * t + 8, :]
            word = ((a >> sh) | (b & keep)) if odd else ((a & keep) | (b << sh))
            word = jnp.transpose(word, (1, 0, 2))
            for r in range(8):
                wqkv_v[(2 * (8 * t + r) + odd) * 3 + j, pl.ds(j0, 8), :] = word[r]

        pieces = [(j, g, t, odd) for j in range(3) for g in range(db // 16)
                  for t in range(H // 16) for odd in range(2)]

        r0 = pl.multiple_of(i * _TB, _TB)
        pre = _matmul(pltpu.bitcast(la_v[...], _BF16), w3_v)
        for z in _anchors(pre, len(pieces), zero):
            relayout(*pieces.pop(), z)
        y = x1_v[pl.ds(r0, _TB), :] + _matmul(_gelu(pre).astype(_BF16), w4_v)
        nxt = jnp.minimum(i + 1, n_blk - 1) * _TB
        rows = 32
        for g, z in enumerate(_anchors(y[:, :D // 2], _TB // rows, zero)):
            norm3(pl.multiple_of(nxt + g * rows, rows), g * rows, rows, z)
        hb_v[pl.ds(r0 + _PAD, _TB), :] = y * jax.nn.sigmoid(y)
        return carry

    jax.lax.fori_loop(0, n_blk, phase_r, 0)

    w_wait(4)
    wo_u = wo_v.bitcast(_U32)
    mem0_copy.wait()
    h_v[0:M, :] = mem0_v[...].astype(_F32)
    h_early = H - H // 4

    def proj(h, j):
        return _dot(h_v[...], pltpu.bitcast(wqkv_v[h * 3 + j], _BF16))

    def out_proj(n, h0, h1):
        w = wo_u[n, h0 * (_LANES // 2):h1 * (_LANES // 2), :]
        return _dot(o_v[:, h0 * _LANES:h1 * _LANES], pltpu.bitcast(w, _BF16))

    def step(s, carry):
        r0 = pl.multiple_of(s * seg, seg)
        h_v[M:L, :] = xn_v[pl.ds(r0, seg), :]
        qi = jax.lax.broadcasted_iota(jnp.int32, (L, L), 0)
        ki = jax.lax.broadcasted_iota(jnp.int32, (L, L), 1)
        mask = (qi < M) | (qi >= ki)
        qkv, prob = {}, {}

        def scores(h):
            q, k, _ = qkv[h]
            sc = jax.lax.dot_general(q, k, (((1,), (1,)), ((), ())),
                                     preferred_element_type=_F32)
            sc = jnp.where(mask, sc * scale, -1000000000.0)
            p = jnp.exp(sc - jnp.max(sc, axis=-1, keepdims=True))
            prob[h] = p / jnp.sum(p, axis=-1, keepdims=True)

        def values(h):
            o_v[:, h * _LANES:(h + 1) * _LANES] = _dot(prob.pop(h), qkv.pop(h)[2])

        for t in range(H + n_col):
            if t < H:
                qkv[t] = (proj(t, 0), proj(t, 1), proj(t, 2))
            else:
                n = t - H
                acc_v[:, n * _LANES:(n + 1) * _LANES] = out_proj(n, 0, h_early)
            if 0 <= t - _LAG_S < H:
                scores(t - _LAG_S)
            if 0 <= t - _LAG_V < H:
                values(t - _LAG_V)

        for n in range(n_col):
            cols = slice(n * _LANES, (n + 1) * _LANES)
            o = acc_v[:, cols] + out_proj(n, h_early, H)
            h_v[0:M, cols] = o[0:M]
            res = (x_v[pl.ds(r0, seg), cols].astype(_F32)
                   + o[M:L] * hb_v[pl.ds(r0 + _PAD, seg), cols])
            x_v[pl.ds(r0, seg), cols] = res.astype(x_v.dtype)
        out_copy(s).start()
        return carry

    jax.lax.fori_loop(0, n_seg, step, 0, unroll=2)
    pltpu.make_async_copy(x_v, out_hbm, sem_io.at[0]).wait()


@functools.partial(jax.jit, static_argnames=("A_seg_len",))
def pallas_recurrent_scan__memory_aug_recurrent_mem_tr__mixer_s_mlp__prompt_kernel(
    A_x, A_mem0, A_Wq, A_Wk, A_Wv, A_Wo, A_seg_len, B_x, B_w1, B_w2, B_w3, B_w4,
):
    del B_x
    B, S, D = A_x.shape
    M = A_mem0.shape[1]
    _, H, Dh = A_Wq.shape
    F = B_w3.shape[1]
    seg = int(A_seg_len)
    n_blk = S // _TB
    n_col = D // _LANES
    assert B == 1 and Dh == _LANES and S % (2 * _TB) == 0 and n_blk >= 4
    assert S % (2 * seg) == 0 and seg % 16 == 0 and M % 8 == 0 and M + seg <= _LANES
    assert H % 16 == 0 and D % (16 * n_blk) == 0 and _LAG_V <= min(n_col, H // 4)

    out = pl.pallas_call(
        functools.partial(_kernel, seg=seg, n_heads=H),
        out_shape=jax.ShapeDtypeStruct((S, D), A_x.dtype),
        in_specs=[pl.BlockSpec(memory_space=pl.ANY)] * 10,
        out_specs=pl.BlockSpec(memory_space=pl.ANY),
        scratch_shapes=[
            pltpu.VMEM((S, D), _BF16),
            pltpu.VMEM((S, D), _F32),
            pltpu.VMEM((S + 2 * _PAD, D), _F32),
            pltpu.VMEM((S, D), _F32),
            pltpu.VMEM((_TB // 2, D), _U32),
            pltpu.VMEM((_TB // 2, D), _U32),
            pltpu.VMEM((3 * H, D // 2, Dh), _U32),
            pltpu.VMEM((n_col, H * Dh, _LANES), _BF16),
            pltpu.VMEM((n_col, D, _LANES), _BF16),
            pltpu.VMEM((n_col, D, _LANES), _BF16),
            pltpu.VMEM((F // _LANES, D, _LANES), _BF16),
            pltpu.VMEM((n_col, F, _LANES), _BF16),
            pltpu.VMEM((6, (D // n_blk) * H, Dh), _BF16),
            pltpu.VMEM((M + seg, D), _F32),
            pltpu.VMEM((M + seg, H * Dh), _F32),
            pltpu.VMEM((M + seg, D), _F32),
            pltpu.VMEM((M, D), _BF16),
            pltpu.SemaphoreType.DMA((n_blk,)),
            pltpu.SemaphoreType.DMA((5,)),
            pltpu.SemaphoreType.DMA((6,)),
            pltpu.SemaphoreType.DMA((2,)),
        ],
        compiler_params=pltpu.CompilerParams(vmem_limit_bytes=120 * 1024 * 1024),
    )(
        A_x.reshape(S, D), A_mem0.reshape(M, D),
        A_Wq.reshape(D * H, Dh), A_Wk.reshape(D * H, Dh), A_Wv.reshape(D * H, Dh),
        A_Wo.reshape(H * Dh, D), B_w1, B_w2, B_w3, B_w4,
    )
    return out.reshape(B, S, D)
```

```python
import functools

import jax
import jax.numpy as jnp
from jax.experimental import pallas as pl
from jax.experimental.pallas import tpu as pltpu

_EPS = 1e-05
_LANES = 128
_PAD = 8
_TB = 256
_HB = _TB // 2
_LAG_S = 1
_LAG_V = 3
_F32 = jnp.float32
_BF16 = jnp.bfloat16
_U32 = jnp.uint32


def _layernorm(x):
    m = jnp.mean(x, axis=-1, keepdims=True)
    d = x - m
    v = jnp.mean(d * d, axis=-1, keepdims=True)
    return d * jax.lax.rsqrt(v + _EPS)


def _gelu(x):
    return jax.nn.gelu(x, approximate=True)


def _dot(a, b):
    return jnp.dot(a, b, preferred_element_type=_F32)


def _strassen_lhs(a11, a12, a21, a22):
    return [a11 + a22, a21 + a22, a11, a22, a11 + a12, a21 - a11, a12 - a22]


def _strassen_rhs(b11, b12, b21, b22):
    return [b11 + b22, b11, b12 - b22, b21 - b11, b22, b11 + b12, b21 + b22]


def _strassen_out(m):
    return (m[0] + m[3] - m[4] + m[6], m[2] + m[4], m[1] + m[3], m[0] - m[1] + m[2] + m[5])


def _halves(top, bottom):
    k = top.shape[1] // 2
    return top[:, :k], top[:, k:], bottom[:, :k], bottom[:, k:]


def _anchors(tiles, count, zero):
    per = -(-count // len(tiles))
    out = []
    for p in range(count):
        n, r = divmod(p * len(tiles) * per // count, per)
        r0 = r * (tiles[n].shape[0] // per) // 8 * 8
        out.append(pltpu.bitcast(tiles[n][r0:r0 + 8], _U32) & zero)
    return out


def _token(values, zero):
    bits = [pltpu.bitcast(v[r:r + 8, c:c + _LANES], _U32) for v in values
            for r in range(0, v.shape[0], 8) for c in range(0, v.shape[1], _LANES)]
    return functools.reduce(jnp.bitwise_or, bits) & zero


def _kernel(x_hbm, mem0_hbm, wq_hbm, wk_hbm, wv_hbm, wo_hbm, w1_hbm, w2_hbm, w3_hbm, w4_hbm,
            out_hbm,
            x_v, xn_v, hb_v, x1_v, la_u, lb_u, wa_u, wb_u, wqkv_u, wo_v, stage_v,
            h_v, o_v, acc_v, mem0_v,
            sem_x, sem_w, sem_st, sem_io,
            *, seg, n_heads):
    S, D = x_v.shape
    M = mem0_v.shape[0]
    L = M + seg
    H = n_heads
    n_blk = S // _TB
    n_seg = S // seg
    n_col = D // _LANES
    db = D // n_blk
    c = D // 4
    scale = _LANES ** (-0.5)

    w_hbm = (w1_hbm, w2_hbm, w3_hbm, w4_hbm)
    w_u = (wa_u, wa_u, wb_u, wb_u)

    def w_start(j, part=0, parts=1):
        src, dst = w_hbm[j], w_u[j].bitcast(_BF16)
        kh, nh = src.shape[0] // 2, src.shape[1] // 2
        todo = [(n, r, q) for n in range(nh // _LANES) for r in range(2) for q in range(2)]
        for n, r, q in todo[part * len(todo) // parts:(part + 1) * len(todo) // parts]:
            pltpu.make_async_copy(
                src.at[pl.ds(r * kh, kh), pl.ds(q * nh + n * _LANES, _LANES)],
                dst.at[1 + 2 * r + q, pl.ds((j % 2) * dst.shape[1] // 2 + n * kh, kh)],
                sem_w.at[j]).start(priority=min(j, 1))

    def w_wait(j):
        dst = w_u[j].bitcast(_BF16)
        dst = dst.at[pl.ds(1, 4), pl.ds((j % 2) * dst.shape[1] // 2, dst.shape[1] // 2)]
        pltpu.make_async_copy(dst, dst, sem_w.at[j]).wait()

    def w_combine(ref, word0, z=None):
        rows = pl.ds(pl.multiple_of(word0, 8), 8)
        words = [ref[k, rows, :] if z is None else ref[k, rows, :] | z for k in (1, 2, 3, 4)]
        even, odd = (
            _strassen_rhs(*(pltpu.unpack_elementwise(w, index=e, packed_dtype=_BF16,
                                                     unpacked_dtype=_F32) for w in words))
            for e in range(2))
        for k in (0, 2, 3, 5, 6):
            ref[k, rows, :] = pltpu.pack_elementwise([even[k], odd[k]], packed_dtype=_BF16)

    def w_combine_all(j):
        words = w_u[j].shape[1] // 2

        def body(i, carry):
            for g in range(8):
                w_combine(w_u[j], (j % 2) * words + (i * 8 + g) * 8)
            return carry

        jax.lax.fori_loop(0, words // 64, body, 0)

    def products(lhs, j, order=range(7), after=None):
        kh, nh = w_hbm[j].shape[0] // 2, w_hbm[j].shape[1] // 2
        word0 = (j % 2) * w_u[j].shape[1] // 2
        for n in range(nh // _LANES):
            rows = slice(word0 + n * kh // 2, word0 + (n + 1) * kh // 2)
            m = {}
            for k in order:
                w = w_u[j][k, rows, :]
                if after and 7 * n + k in after:
                    w = jnp.concatenate([w[:8] | after[7 * n + k], w[8:]], axis=0)
                m[k] = _dot(lhs[k], pltpu.bitcast(w, _BF16))
            yield [m[k] for k in range(7)]

    def block_of(r0, n, q):
        c0 = (q % 2) * (D // 2) + n * _LANES
        return pl.ds(r0 + (q // 2) * _HB, _HB), slice(c0, c0 + _LANES)

    def put_lhs(dst_u, row0, top, bottom):
        ops = _strassen_lhs(*_halves(top, bottom))
        for k, v in enumerate(ops):
            dst_u.bitcast(_BF16)[pl.ds(k * _HB + row0, top.shape[0]), :] = v.astype(_BF16)
        return [ops[0], ops[5], ops[6]]

    def get_lhs(src_u):
        return [src_u.bitcast(_BF16)[k * _HB:(k + 1) * _HB, :] for k in range(7)]

    def x_copy(i):
        rows = pl.ds(pl.multiple_of(i * _TB, _TB), _TB)
        return pltpu.make_async_copy(x_hbm.at[rows], x_v.at[rows], sem_x.at[i])

    def wo_start(part, parts):
        for n in range(part * n_col // parts, (part + 1) * n_col // parts):
            pltpu.make_async_copy(wo_hbm.at[:, pl.ds(n * _LANES, _LANES)], wo_v.at[n],
                                  sem_w.at[4]).start()

    def stage_copy(i, j):
        src = (wq_hbm, wk_hbm, wv_hbm)[j]
        rows = pl.ds(pl.multiple_of(i * (db * H), db * H), db * H)
        slot = (i % 2) * 3 + j
        return pltpu.make_async_copy(src.at[rows], stage_v.at[slot], sem_st.at[slot])

    def stage_start(i):
        for j in range(3):
            stage_copy(i, j).start()

    def out_copy(s):
        rows = pl.ds(pl.multiple_of(s * seg, seg), seg)
        return pltpu.make_async_copy(x_v.at[rows], out_hbm.at[rows], sem_io.at[0])

    mem0_copy = pltpu.make_async_copy(mem0_hbm, mem0_v, sem_io.at[1])

    def paced(i, plan):
        for k, jobs in enumerate(plan):
            if jobs:
                @pl.when(i == k)
                def _(jobs=jobs):
                    for job, *args in jobs:
                        job(*args)

    plan_p = [[(w_start, 1)],
              [(w_start, 2, 0, 2)],
              [(w_start, 2, 1, 2)],
              [(w_start, 3, 0, 2)]]
    plan_q = [[(w_start, 3, 1, 2)], [], [(stage_start, 0)], []] + [
        [(wo_start, k, 4)] for k in range(4)]

    x_copy(0).start()
    w_start(0)
    x_copy(1).start()
    x_copy(2).start()
    hb_v[0:_PAD, :] = jnp.zeros((_PAD, D), _F32)
    hb_v[_PAD + S:, :] = jnp.zeros((_PAD, D), _F32)

    def norms(dst_u, src0, dst0, rows):
        ln = []
        for r in (0, _HB):
            xn = _layernorm(x_v[pl.ds(src0 + r, rows), :].astype(_F32))
            xn_v[pl.ds(src0 + r, rows), :] = xn
            ln.append(_layernorm(xn))
        return put_lhs(dst_u, dst0, *ln)

    def next_block(fn, blk, first, last, zero):
        nxt = jnp.minimum(blk + 1, n_blk - 1) * _TB
        groups = _HB // 16
        return {first + g * (last - first) // (groups - 1):
                _token(fn(pl.multiple_of(nxt + g * 16, 16), g * 16, 16), zero)
                for g in range(groups)}

    x_copy(0).wait()
    norms(la_u, 0, 0, _HB)
    mem0_copy.start()
    w_wait(0)
    w_combine_all(0)

    def phase_p(i, carry):
        paced(i, plan_p)
        for k in (3, 4):
            @pl.when(2 * i + k < n_blk)
            def _(k=k):
                x_copy(2 * i + k).start()

        x_copy(2 * i + 1).wait()

        @pl.when(2 * i + 2 < n_blk)
        def _():
            x_copy(2 * i + 2).wait()

        zero = pltpu.bitcast(hb_v[0:8, 0:_LANES], _U32)
        for k, (cur_u, nxt_u) in enumerate(((la_u, lb_u), (lb_u, la_u))):
            blk = 2 * i + k
            r0 = pl.multiple_of(blk * _TB, _TB)
            after = next_block(functools.partial(norms, nxt_u), blk, 7, 27, zero)
            for n, m in enumerate(products(get_lhs(cur_u), 0, after=after)):
                for q, v in enumerate(_strassen_out(m)):
                    hb_v[block_of(r0 + _PAD, n, q)] = _gelu(v)
        return carry

    jax.lax.fori_loop(0, n_blk // 2, phase_p, 0)

    w_wait(1)
    w_combine_all(1)
    w_wait(2)

    def phase_q(i, carry):
        paced(i, plan_q)

        @pl.when(i == n_blk // 2)
        def _():
            w_wait(3)

        zero = pltpu.bitcast(hb_v[0:8, 0:_LANES], _U32)
        r0 = pl.multiple_of(i * _TB, _TB)
        parts = []
        for q, shift in enumerate((-1, 1, -2, 2)):
            win = hb_v[pl.ds(r0, _TB + 2 * _PAD), q * c:(q + 1) * c]
            parts.append(win[_PAD + shift:_PAD + shift + _TB])
        g = jnp.concatenate(parts, axis=1)
        seen = []
        lhs = [v.astype(_BF16) for v in _strassen_lhs(*_halves(g[:_HB], g[_HB:]))]
        order = (2, 3, 4, 6, 0, 5, 1)
        for n, m in enumerate(products(lhs, 1, order)):
            seen += [m[k] for k in order]
            for q, v in enumerate(_strassen_out(m)):
                x1_v[block_of(r0, n, q)] = xn_v[block_of(r0, n, q)] + v
        words = wb_u.shape[1] // n_blk
        for p, z in enumerate(_anchors(seen[7:-1], words // 8, zero)):
            w_combine(wb_u, i * words + p * 8, z)
        return carry

    jax.lax.fori_loop(0, n_blk, phase_q, 0)

    def norm3(src0, dst0, rows):
        return put_lhs(la_u, dst0,
                       *(_layernorm(x1_v[pl.ds(src0 + r, rows), :]) for r in (0, _HB)))

    norm3(0, 0, _HB)
    stage_u = stage_v.bitcast(_U32)

    def phase_r(i, carry):
        @pl.when(i + 1 < n_blk)
        def _():
            stage_start(i + 1)

        for j in range(3):
            stage_copy(i, j).wait()

        zero = pltpu.bitcast(hb_v[0:8, 0:_LANES], _U32)

        def relayout(j, g, t, odd, z):
            keep, sh = z | _U32(0xFFFF0000 if odd else 0xFFFF), z | _U32(16)
            j0 = pl.multiple_of(i * (db // 2) + g * 8, 8)
            w = stage_u[(i % 2) * 3 + j, g * 8 * H:(g + 1) * 8 * H, :].reshape(8, H, _LANES)
            a = w[:, 8 * t:8 * t + 8, :]
            b = w[:, H // 2 + 8 * t:H // 2 + 8 * t + 8, :]
            word = ((a >> sh) | (b & keep)) if odd else ((a & keep) | (b << sh))
            word = jnp.transpose(word, (1, 0, 2))
            for r in range(8):
                wqkv_u[(2 * (8 * t + r) + odd) * 3 + j, pl.ds(j0, 8), :] = word[r]

        r0 = pl.multiple_of(i * _TB, _TB)
        seen, ups = [], []
        for m in products(get_lhs(la_u), 2):
            seen += m[:4]
            ups.append(_strassen_lhs(*(_gelu(v) for v in _strassen_out(m))))
        pieces = [(j, g, t, odd) for j in range(3) for g in range(db // 16)
                  for t in range(H // 16) for odd in range(2)]
        for piece, z in zip(pieces, _anchors(seen, len(pieces), zero)):
            relayout(*piece, z)

        lhs = [jnp.concatenate([u[k] for u in ups], axis=1).astype(_BF16) for k in range(7)]
        after = next_block(norm3, i, 2, 16, zero)
        for n, m in enumerate(products(lhs, 3, after=after)):
            for q, v in enumerate(_strassen_out(m)):
                y = x1_v[block_of(r0, n, q)] + v
                hb_v[block_of(r0 + _PAD, n, q)] = y * jax.nn.sigmoid(y)
        return carry

    jax.lax.fori_loop(0, n_blk, phase_r, 0)

    pltpu.make_async_copy(wo_v, wo_v, sem_w.at[4]).wait()
    wo_u = wo_v.bitcast(_U32)
    mem0_copy.wait()
    h_v[0:M, :] = mem0_v[...].astype(_F32)
    h_early = H - H // 4

    def proj(h, j):
        return _dot(h_v[...], pltpu.bitcast(wqkv_u[h * 3 + j], _BF16))

    def out_proj(n, h0, h1):
        w = wo_u[n, h0 * (_LANES // 2):h1 * (_LANES // 2), :]
        return _dot(o_v[:, h0 * _LANES:h1 * _LANES], pltpu.bitcast(w, _BF16))

    def step(s, carry):
        r0 = pl.multiple_of(s * seg, seg)
        h_v[M:L, :] = xn_v[pl.ds(r0, seg), :]
        qi = jax.lax.broadcasted_iota(jnp.int32, (L, L), 0)
        ki = jax.lax.broadcasted_iota(jnp.int32, (L, L), 1)
        mask = (qi < M) | (qi >= ki)
        qkv, prob = {}, {}

        def scores(h):
            q, k, _ = qkv[h]
            sc = jax.lax.dot_general(q, k, (((1,), (1,)), ((), ())),
                                     preferred_element_type=_F32)
            sc = jnp.where(mask, sc * scale, -1000000000.0)
            p = jnp.exp(sc - jnp.max(sc, axis=-1, keepdims=True))
            prob[h] = p / jnp.sum(p, axis=-1, keepdims=True)

        def values(h):
            o_v[:, h * _LANES:(h + 1) * _LANES] = _dot(prob.pop(h), qkv.pop(h)[2])

        for t in range(H + n_col):
            if t < H:
                qkv[t] = (proj(t, 0), proj(t, 1), proj(t, 2))
            else:
                n = t - H
                acc_v[:, n * _LANES:(n + 1) * _LANES] = out_proj(n, 0, h_early)
            if 0 <= t - _LAG_S < H:
                scores(t - _LAG_S)
            if 0 <= t - _LAG_V < H:
                values(t - _LAG_V)

        for n in range(n_col):
            cols = slice(n * _LANES, (n + 1) * _LANES)
            o = acc_v[:, cols] + out_proj(n, h_early, H)
            h_v[0:M, cols] = o[0:M]
            res = (x_v[pl.ds(r0, seg), cols].astype(_F32)
                   + o[M:L] * hb_v[pl.ds(r0 + _PAD, seg), cols])
            x_v[pl.ds(r0, seg), cols] = res.astype(x_v.dtype)
        out_copy(s).start()
        return carry

    jax.lax.fori_loop(0, n_seg, step, 0, unroll=2)
    pltpu.make_async_copy(x_v, out_hbm, sem_io.at[0]).wait()


@functools.partial(jax.jit, static_argnames=("A_seg_len",))
def pallas_recurrent_scan__memory_aug_recurrent_mem_tr__mixer_s_mlp__prompt_kernel(
    A_x, A_mem0, A_Wq, A_Wk, A_Wv, A_Wo, A_seg_len, B_x, B_w1, B_w2, B_w3, B_w4,
):
    del B_x
    B, S, D = A_x.shape
    M = A_mem0.shape[1]
    _, H, Dh = A_Wq.shape
    F = B_w3.shape[1]
    seg = int(A_seg_len)
    n_blk = S // _TB
    n_col = D // _LANES
    assert B == 1 and Dh == _LANES and S % (2 * _TB) == 0 and n_blk >= 8
    assert S % (2 * seg) == 0 and seg % 16 == 0 and M % 8 == 0 and M + seg <= _LANES
    assert H % 16 == 0 and D % (16 * n_blk) == 0 and _LAG_V <= min(n_col, H // 4)
    assert D % 512 == 0 and F % 256 == 0 and (D * F) % (32 * _LANES * n_blk) == 0

    out = pl.pallas_call(
        functools.partial(_kernel, seg=seg, n_heads=H),
        out_shape=jax.ShapeDtypeStruct((S, D), A_x.dtype),
        in_specs=[pl.BlockSpec(memory_space=pl.ANY)] * 10,
        out_specs=pl.BlockSpec(memory_space=pl.ANY),
        scratch_shapes=[
            pltpu.VMEM((S, D), _BF16),
            pltpu.VMEM((S, D), _F32),
            pltpu.VMEM((S + 2 * _PAD, D), _F32),
            pltpu.VMEM((S, D), _F32),
            pltpu.VMEM((7 * _HB // 2, D // 2), _U32),
            pltpu.VMEM((7 * _HB // 2, D // 2), _U32),
            pltpu.VMEM((7, D * D // (4 * _LANES), _LANES), _U32),
            pltpu.VMEM((7, D * F // (4 * _LANES), _LANES), _U32),
            pltpu.VMEM((3 * H, D // 2, Dh), _U32),
            pltpu.VMEM((n_col, H * Dh, _LANES), _BF16),
            pltpu.VMEM((6, (D // n_blk) * H, Dh), _BF16),
            pltpu.VMEM((M + seg, D), _F32),
            pltpu.VMEM((M + seg, H * Dh), _F32),
            pltpu.VMEM((M + seg, D), _F32),
            pltpu.VMEM((M, D), _BF16),
            pltpu.SemaphoreType.DMA((n_blk,)),
            pltpu.SemaphoreType.DMA((5,)),
            pltpu.SemaphoreType.DMA((6,)),
            pltpu.SemaphoreType.DMA((2,)),
        ],
        compiler_params=pltpu.CompilerParams(vmem_limit_bytes=120 * 1024 * 1024),
    )(
        A_x.reshape(S, D), A_mem0.reshape(M, D),
        A_Wq.reshape(D * H, Dh), A_Wk.reshape(D * H, Dh), A_Wv.reshape(D * H, Dh),
        A_Wo.reshape(H * Dh, D), B_w1, B_w2, B_w3, B_w4,
    )
    return out.reshape(B, S, D)
```

```python
import functools

import jax
import jax.numpy as jnp
from jax.experimental import pallas as pl
from jax.experimental.pallas import tpu as pltpu

_EPS = 1e-05
_LANES = 128
_PAD = 8
_TB = 256
_HB = _TB // 2
_LAG_S = 1
_LAG_V = 3
_F32 = jnp.float32
_BF16 = jnp.bfloat16
_U32 = jnp.uint32


def _layernorm(x):
    m = jnp.mean(x, axis=-1, keepdims=True)
    d = x - m
    v = jnp.mean(d * d, axis=-1, keepdims=True)
    return d * jax.lax.rsqrt(v + _EPS)


def _gelu(x):
    return jax.nn.gelu(x, approximate=True)


def _dot(a, b):
    return jnp.dot(a, b, preferred_element_type=_F32)


def _strassen_lhs(a11, a12, a21, a22):
    return [a11 + a22, a21 + a22, a11, a22, a11 + a12, a21 - a11, a12 - a22]


def _strassen_rhs(b11, b12, b21, b22):
    return [b11 + b22, b11, b12 - b22, b21 - b11, b22, b11 + b12, b21 + b22]


def _strassen_out(m):
    return (m[0] + m[3] - m[4] + m[6], m[2] + m[4], m[1] + m[3], m[0] - m[1] + m[2] + m[5])


def _halves(top, bottom):
    k = top.shape[1] // 2
    return top[:, :k], top[:, k:], bottom[:, :k], bottom[:, k:]


def _anchors(tiles, count, zero):
    per = -(-count // len(tiles))
    out = []
    for p in range(count):
        n, r = divmod(p * len(tiles) * per // count, per)
        r0 = r * (tiles[n].shape[0] // per) // 8 * 8
        out.append(pltpu.bitcast(tiles[n][r0:r0 + 8], _U32) & zero)
    return out


def _token(values, zero):
    bits = [pltpu.bitcast(v[r:r + 8, c:c + _LANES], _U32) for v in values
            for r in range(0, v.shape[0], 8) for c in range(0, v.shape[1], _LANES)]
    return functools.reduce(jnp.bitwise_or, bits) & zero


def _kernel(x_hbm, mem0_hbm, wq_hbm, wk_hbm, wv_hbm, wo_hbm, w1_hbm, w2_hbm, w3_hbm, w4_hbm,
            out_hbm,
            x_v, xn_v, hb_v, x1_v, la_u, lb_u, wa_u, wb_u, wqkv_u, wo_v, stage_v,
            h_v, o_v, acc_v, mem0_v,
            sem_x, sem_w, sem_st, sem_io,
            *, seg, n_heads):
    S, D = x_v.shape
    M = mem0_v.shape[0]
    L = M + seg
    H = n_heads
    n_blk = S // _TB
    n_seg = S // seg
    n_col = D // _LANES
    db = D // n_blk
    c = D // 4
    scale = _LANES ** (-0.5)

    w_hbm = (w1_hbm, w2_hbm, w3_hbm, w4_hbm)
    w_u = (wa_u, wa_u, wb_u, wb_u)

    def w_start(j, part=0, parts=1, priority=0):
        src, dst = w_hbm[j], w_u[j].bitcast(_BF16)
        kh, nh = src.shape[0] // 2, src.shape[1] // 2
        todo = [(n, r, q) for n in range(nh // _LANES) for r in range(2) for q in range(2)]
        for n, r, q in todo[part * len(todo) // parts:(part + 1) * len(todo) // parts]:
            pltpu.make_async_copy(
                src.at[pl.ds(r * kh, kh), pl.ds(q * nh + n * _LANES, _LANES)],
                dst.at[1 + 2 * r + q, pl.ds((j % 2) * dst.shape[1] // 2 + n * kh, kh)],
                sem_w.at[j]).start(priority=priority)

    def w_wait(j):
        dst = w_u[j].bitcast(_BF16)
        dst = dst.at[pl.ds(1, 4), pl.ds((j % 2) * dst.shape[1] // 2, dst.shape[1] // 2)]
        pltpu.make_async_copy(dst, dst, sem_w.at[j]).wait()

    def w_combine(ref, word0, z=None):
        rows = pl.ds(pl.multiple_of(word0, 8), 8)
        words = [ref[k, rows, :] if z is None else ref[k, rows, :] | z for k in (1, 2, 3, 4)]
        even, odd = (
            _strassen_rhs(*(pltpu.unpack_elementwise(w, index=e, packed_dtype=_BF16,
                                                     unpacked_dtype=_F32) for w in words))
            for e in range(2))
        for k in (0, 2, 3, 5, 6):
            ref[k, rows, :] = pltpu.pack_elementwise([even[k], odd[k]], packed_dtype=_BF16)

    def w_combine_all(j):
        words = w_u[j].shape[1] // 2

        def body(i, carry):
            for g in range(8):
                w_combine(w_u[j], (j % 2) * words + (i * 8 + g) * 8)
            return carry

        jax.lax.fori_loop(0, words // 64, body, 0)

    def products(lhs, j, order=range(7), after=None):
        kh, nh = w_hbm[j].shape[0] // 2, w_hbm[j].shape[1] // 2
        word0 = (j % 2) * w_u[j].shape[1] // 2
        for n in range(nh // _LANES):
            rows = slice(word0 + n * kh // 2, word0 + (n + 1) * kh // 2)
            m = {}
            for k in order:
                w = w_u[j][k, rows, :]
                if after and 7 * n + k in after:
                    w = jnp.concatenate([w[:8] | after[7 * n + k], w[8:]], axis=0)
                m[k] = _dot(lhs[k], pltpu.bitcast(w, _BF16))
            yield [m[k] for k in range(7)]

    def block_of(r0, n, q):
        c0 = (q % 2) * (D // 2) + n * _LANES
        return pl.ds(r0 + (q // 2) * _HB, _HB), slice(c0, c0 + _LANES)

    def put_lhs(dst_u, row0, top, bottom):
        ops = _strassen_lhs(*_halves(top, bottom))
        for k, v in enumerate(ops):
            dst_u.bitcast(_BF16)[pl.ds(k * _HB + row0, top.shape[0]), :] = v.astype(_BF16)
        return [ops[0], ops[5], ops[6]]

    def get_lhs(src_u):
        return [src_u.bitcast(_BF16)[k * _HB:(k + 1) * _HB, :] for k in range(7)]

    def x_copy(i):
        rows = pl.ds(pl.multiple_of(i * _TB, _TB), _TB)
        return pltpu.make_async_copy(x_hbm.at[rows], x_v.at[rows], sem_x.at[i])

    def wo_start(part, parts):
        for n in range(part * n_col // parts, (part + 1) * n_col // parts):
            pltpu.make_async_copy(wo_hbm.at[:, pl.ds(n * _LANES, _LANES)], wo_v.at[n],
                                  sem_w.at[4]).start()

    def stage_copy(i, j):
        src = (wq_hbm, wk_hbm, wv_hbm)[j]
        rows = pl.ds(pl.multiple_of(i * (db * H), db * H), db * H)
        slot = (i % 2) * 3 + j
        return pltpu.make_async_copy(src.at[rows], stage_v.at[slot], sem_st.at[slot])

    def stage_start(i):
        for j in range(3):
            stage_copy(i, j).start()

    def out_copy(s):
        rows = pl.ds(pl.multiple_of(s * seg, seg), seg)
        return pltpu.make_async_copy(x_v.at[rows], out_hbm.at[rows], sem_io.at[0])

    mem0_copy = pltpu.make_async_copy(mem0_hbm, mem0_v, sem_io.at[1])

    def paced(i, plan):
        for k, jobs in enumerate(plan):
            if jobs:
                @pl.when(i == k)
                def _(jobs=jobs):
                    for job, *args in jobs:
                        job(*args)

    plan_p = [[(w_start, 1, 0, 1, 1), (w_start, 2, 0, 3, 1)],
              [(w_start, 2, 1, 3, 1)],
              [(w_start, 2, 2, 3, 1)],
              [(w_start, 3, 0, 2, 1)]]
    plan_q = [[(w_start, 3, 1, 2)], [], [], [(stage_start, 0)]] + [
        [(wo_start, k, 4)] for k in range(4)]

    x_copy(0).start()
    w_start(0)
    x_copy(1).start()
    x_copy(2).start()
    hb_v[0:_PAD, :] = jnp.zeros((_PAD, D), _F32)
    hb_v[_PAD + S:, :] = jnp.zeros((_PAD, D), _F32)

    def norms(dst_u, src0, dst0, rows):
        ln = []
        for r in (0, _HB):
            xn = _layernorm(x_v[pl.ds(src0 + r, rows), :].astype(_F32))
            xn_v[pl.ds(src0 + r, rows), :] = xn
            ln.append(_layernorm(xn))
        return put_lhs(dst_u, dst0, *ln)

    def next_block(fn, blk, first, last, zero):
        nxt = jnp.minimum(blk + 1, n_blk - 1) * _TB
        groups = _HB // 16
        return {first + g * (last - first) // (groups - 1):
                _token(fn(pl.multiple_of(nxt + g * 16, 16), g * 16, 16), zero)
                for g in range(groups)}

    x_copy(0).wait()
    norms(la_u, 0, 0, _HB)
    mem0_copy.start()
    w_wait(0)
    w_combine_all(0)

    def phase_p(i, carry):
        paced(i, plan_p)
        for k in (3, 4):
            @pl.when(2 * i + k < n_blk)
            def _(k=k):
                x_copy(2 * i + k).start()

        x_copy(2 * i + 1).wait()

        @pl.when(2 * i + 2 < n_blk)
        def _():
            x_copy(2 * i + 2).wait()

        zero = pltpu.bitcast(hb_v[0:8, 0:_LANES], _U32)
        for k, (cur_u, nxt_u) in enumerate(((la_u, lb_u), (lb_u, la_u))):
            blk = 2 * i + k
            r0 = pl.multiple_of(blk * _TB, _TB)
            after = next_block(functools.partial(norms, nxt_u), blk, 7, 27, zero)
            for n, m in enumerate(products(get_lhs(cur_u), 0, after=after)):
                for q, v in enumerate(_strassen_out(m)):
                    hb_v[block_of(r0 + _PAD, n, q)] = _gelu(v)
        return carry

    jax.lax.fori_loop(0, n_blk // 2, phase_p, 0)

    w_wait(1)
    w_combine_all(1)
    w_wait(2)

    def phase_q(i, carry):
        paced(i, plan_q)

        @pl.when(i == n_blk // 2)
        def _():
            w_wait(3)

        zero = pltpu.bitcast(hb_v[0:8, 0:_LANES], _U32)
        r0 = pl.multiple_of(i * _TB, _TB)
        parts = []
        for q, shift in enumerate((-1, 1, -2, 2)):
            win = hb_v[pl.ds(r0, _TB + 2 * _PAD), q * c:(q + 1) * c]
            parts.append(win[_PAD + shift:_PAD + shift + _TB])
        g = jnp.concatenate(parts, axis=1)
        seen = []
        lhs = [v.astype(_BF16) for v in _strassen_lhs(*_halves(g[:_HB], g[_HB:]))]
        order = (2, 3, 4, 6, 0, 5, 1)
        for n, m in enumerate(products(lhs, 1, order)):
            seen += [m[k] for k in order]
            for q, v in enumerate(_strassen_out(m)):
                x1_v[block_of(r0, n, q)] = xn_v[block_of(r0, n, q)] + v
        words = wb_u.shape[1] // n_blk
        for p, z in enumerate(_anchors(seen[7:-1], words // 8, zero)):
            w_combine(wb_u, i * words + p * 8, z)
        return carry

    jax.lax.fori_loop(0, n_blk, phase_q, 0)

    def norm3(src0, dst0, rows):
        return put_lhs(la_u, dst0,
                       *(_layernorm(x1_v[pl.ds(src0 + r, rows), :]) for r in (0, _HB)))

    norm3(0, 0, _HB)
    stage_u = stage_v.bitcast(_U32)

    def phase_r(i, carry):
        @pl.when(i + 1 < n_blk)
        def _():
            stage_start(i + 1)

        for j in range(3):
            stage_copy(i, j).wait()

        zero = pltpu.bitcast(hb_v[0:8, 0:_LANES], _U32)

        def relayout(j, g, t, odd, z):
            keep, sh = z | _U32(0xFFFF0000 if odd else 0xFFFF), z | _U32(16)
            j0 = pl.multiple_of(i * (db // 2) + g * 8, 8)
            w = stage_u[(i % 2) * 3 + j, g * 8 * H:(g + 1) * 8 * H, :].reshape(8, H, _LANES)
            a = w[:, 8 * t:8 * t + 8, :]
            b = w[:, H // 2 + 8 * t:H // 2 + 8 * t + 8, :]
            word = ((a >> sh) | (b & keep)) if odd else ((a & keep) | (b << sh))
            word = jnp.transpose(word, (1, 0, 2))
            for r in range(8):
                wqkv_u[(2 * (8 * t + r) + odd) * 3 + j, pl.ds(j0, 8), :] = word[r]

        r0 = pl.multiple_of(i * _TB, _TB)
        seen, ups = [], []
        for m in products(get_lhs(la_u), 2):
            seen += m[:4]
            ups.append(_strassen_lhs(*(_gelu(v) for v in _strassen_out(m))))
        pieces = [(j, g, t, odd) for j in range(3) for g in range(db // 16)
                  for t in range(H // 16) for odd in range(2)]
        for piece, z in zip(pieces, _anchors(seen, len(pieces), zero)):
            relayout(*piece, z)

        lhs = [jnp.concatenate([u[k] for u in ups], axis=1).astype(_BF16) for k in range(7)]
        after = next_block(norm3, i, 2, 16, zero)
        for n, m in enumerate(products(lhs, 3, after=after)):
            for q, v in enumerate(_strassen_out(m)):
                y = x1_v[block_of(r0, n, q)] + v
                hb_v[block_of(r0 + _PAD, n, q)] = y * jax.nn.sigmoid(y)
        return carry

    jax.lax.fori_loop(0, n_blk, phase_r, 0)

    pltpu.make_async_copy(wo_v, wo_v, sem_w.at[4]).wait()
    wo_u = wo_v.bitcast(_U32)
    mem0_copy.wait()
    h_v[0:M, :] = mem0_v[...].astype(_F32)
    h_early = H - H // 4

    def proj(h, j):
        return _dot(h_v[...], pltpu.bitcast(wqkv_u[h * 3 + j], _BF16))

    def first_proj():
        kh = D // 2
        for j in range(3):
            acc_v[:, j * _LANES:(j + 1) * _LANES] = _dot(
                h_v[:, :kh], pltpu.bitcast(wqkv_u[j, :kh // 2, :], _BF16))
        return tuple(
            acc_v[:, j * _LANES:(j + 1) * _LANES]
            + _dot(h_v[:, kh:], pltpu.bitcast(wqkv_u[j, kh // 2:, :], _BF16)) for j in range(3))

    def out_proj(n, h0, h1):
        w = wo_u[n, h0 * (_LANES // 2):h1 * (_LANES // 2), :]
        return _dot(o_v[:, h0 * _LANES:h1 * _LANES], pltpu.bitcast(w, _BF16))

    def step(s, carry):
        r0 = pl.multiple_of(s * seg, seg)
        h_v[M:L, :] = xn_v[pl.ds(r0, seg), :]
        qi = jax.lax.broadcasted_iota(jnp.int32, (L, L), 0)
        ki = jax.lax.broadcasted_iota(jnp.int32, (L, L), 1)
        mask = (qi < M) | (qi >= ki)
        qkv, prob = {}, {}

        def scores(h):
            q, k, _ = qkv[h]
            sc = jax.lax.dot_general(q, k, (((1,), (1,)), ((), ())),
                                     preferred_element_type=_F32)
            sc = jnp.where(mask, sc * scale, -1000000000.0)
            p = jnp.exp(sc - jnp.max(sc, axis=-1, keepdims=True))
            prob[h] = p / jnp.sum(p, axis=-1, keepdims=True)

        def values(h):
            o_v[:, h * _LANES:(h + 1) * _LANES] = _dot(prob.pop(h), qkv.pop(h)[2])

        for t in range(H + n_col):
            if t == 0:
                qkv[t] = first_proj()
            elif t < H:
                qkv[t] = (proj(t, 0), proj(t, 1), proj(t, 2))
            else:
                n = t - H
                acc_v[:, n * _LANES:(n + 1) * _LANES] = out_proj(n, 0, h_early)
            if 0 <= t - _LAG_S < H:
                scores(t - _LAG_S)
            if 0 <= t - _LAG_V < H:
                values(t - _LAG_V)

        for n in range(n_col):
            cols = slice(n * _LANES, (n + 1) * _LANES)
            o = acc_v[:, cols] + out_proj(n, h_early, H)
            h_v[0:M, cols] = o[0:M]
            res = (x_v[pl.ds(r0, seg), cols].astype(_F32)
                   + o[M:L] * hb_v[pl.ds(r0 + _PAD, seg), cols])
            x_v[pl.ds(r0, seg), cols] = res.astype(x_v.dtype)
        out_copy(s).start()
        return carry

    jax.lax.fori_loop(0, n_seg, step, 0, unroll=2)
    pltpu.make_async_copy(x_v, out_hbm, sem_io.at[0]).wait()


@functools.partial(jax.jit, static_argnames=("A_seg_len",))
def pallas_recurrent_scan__memory_aug_recurrent_mem_tr__mixer_s_mlp__prompt_kernel(
    A_x, A_mem0, A_Wq, A_Wk, A_Wv, A_Wo, A_seg_len, B_x, B_w1, B_w2, B_w3, B_w4,
):
    del B_x
    B, S, D = A_x.shape
    M = A_mem0.shape[1]
    _, H, Dh = A_Wq.shape
    F = B_w3.shape[1]
    seg = int(A_seg_len)
    n_blk = S // _TB
    n_col = D // _LANES
    assert B == 1 and Dh == _LANES and S % (2 * _TB) == 0 and n_blk >= 8
    assert S % (2 * seg) == 0 and seg % 16 == 0 and M % 8 == 0 and M + seg <= _LANES
    assert H % 16 == 0 and D % (16 * n_blk) == 0 and _LAG_V <= min(n_col, H // 4)
    assert D % 512 == 0 and F % 256 == 0 and (D * F) % (32 * _LANES * n_blk) == 0

    out = pl.pallas_call(
        functools.partial(_kernel, seg=seg, n_heads=H),
        out_shape=jax.ShapeDtypeStruct((S, D), A_x.dtype),
        in_specs=[pl.BlockSpec(memory_space=pl.ANY)] * 10,
        out_specs=pl.BlockSpec(memory_space=pl.ANY),
        scratch_shapes=[
            pltpu.VMEM((S, D), _BF16),
            pltpu.VMEM((S, D), _F32),
            pltpu.VMEM((S + 2 * _PAD, D), _F32),
            pltpu.VMEM((S, D), _F32),
            pltpu.VMEM((7 * _HB // 2, D // 2), _U32),
            pltpu.VMEM((7 * _HB // 2, D // 2), _U32),
            pltpu.VMEM((7, D * D // (4 * _LANES), _LANES), _U32),
            pltpu.VMEM((7, D * F // (4 * _LANES), _LANES), _U32),
            pltpu.VMEM((3 * H, D // 2, Dh), _U32),
            pltpu.VMEM((n_col, H * Dh, _LANES), _BF16),
            pltpu.VMEM((6, (D // n_blk) * H, Dh), _BF16),
            pltpu.VMEM((M + seg, D), _F32),
            pltpu.VMEM((M + seg, H * Dh), _F32),
            pltpu.VMEM((M + seg, D), _F32),
            pltpu.VMEM((M, D), _BF16),
            pltpu.SemaphoreType.DMA((n_blk,)),
            pltpu.SemaphoreType.DMA((5,)),
            pltpu.SemaphoreType.DMA((6,)),
            pltpu.SemaphoreType.DMA((2,)),
        ],
        compiler_params=pltpu.CompilerParams(vmem_limit_bytes=120 * 1024 * 1024),
    )(
        A_x.reshape(S, D), A_mem0.reshape(M, D),
        A_Wq.reshape(D * H, Dh), A_Wk.reshape(D * H, Dh), A_Wv.reshape(D * H, Dh),
        A_Wo.reshape(H * Dh, D), B_w1, B_w2, B_w3, B_w4,
    )
    return out.reshape(B, S, D)
```

```python
import functools

import jax
import jax.numpy as jnp
from jax.experimental import pallas as pl
from jax.experimental.pallas import tpu as pltpu

_EPS = 1e-05
_LANES = 128
_PAD = 8
_TB = 256
_LAG_S = 1
_LAG_V = 3
_F32 = jnp.float32
_BF16 = jnp.bfloat16
_U32 = jnp.uint32


def _layernorm(x):
    m = jnp.mean(x, axis=-1, keepdims=True)
    d = x - m
    v = jnp.mean(d * d, axis=-1, keepdims=True)
    return d * jax.lax.rsqrt(v + _EPS)


def _gelu(x):
    return jax.nn.gelu(x, approximate=True)


def _dot(a, b):
    return jnp.dot(a, b, preferred_element_type=_F32)


def _matmul(a, w_v, after=None):
    w = w_v.bitcast(_U32)
    words = 4 * _LANES // 2
    rounds = w.shape[1] // words
    out = []
    for n in range(w_v.shape[0]):
        tile = w[n]
        for r in range(rounds):
            if after and n * rounds + r in after:
                r0 = r * words
                parts = (tile[:r0], tile[r0:r0 + 8] | after[n * rounds + r], tile[r0 + 8:])
                tile = jnp.concatenate([p for p in parts if p.shape[0]], axis=0)
        out.append(_dot(a, pltpu.bitcast(tile, _BF16)))
    return jnp.concatenate(out, axis=1)


def _token(value, zero):
    bits = [pltpu.bitcast(value[r:r + 8, c:c + _LANES], _U32)
            for r in range(0, value.shape[0], 8) for c in range(0, value.shape[1], _LANES)]
    return functools.reduce(jnp.bitwise_or, bits) & zero


def _anchors(val, count, zero):
    cols = val.shape[1] // _LANES
    per = -(-count // cols)
    out = []
    for p in range(count):
        n, r = divmod(p * cols * per // count, per)
        r0 = r * (val.shape[0] // per) // 8 * 8
        out.append(pltpu.bitcast(val[r0:r0 + 8, n * _LANES:(n + 1) * _LANES], _U32) & zero)
    return out


def _kernel(x_hbm, mem0_hbm, wq_hbm, wk_hbm, wv_hbm, wo_hbm, w1_hbm, w2_hbm, w3_hbm, w4_hbm,
            out_hbm,
            x_v, xn_v, hb_v, x1_v, la_v, lb_v, wqkv_v, wo_v, w1_v, w2_v, w3_v, w4_v, stage_v,
            h_v, o_v, acc_v, mem0_v,
            sem_x, sem_w, sem_st, sem_io,
            *, seg, n_heads):
    S, D = x_v.shape
    M = mem0_v.shape[0]
    L = M + seg
    H = n_heads
    n_blk = S // _TB
    n_seg = S // seg
    n_col = D // _LANES
    db = D // n_blk
    c = D // 4
    scale = _LANES ** (-0.5)

    def x_copy(i):
        rows = pl.ds(pl.multiple_of(i * _TB, _TB), _TB)
        return pltpu.make_async_copy(x_hbm.at[rows], x_v.at[rows], sem_x.at[i])

    w_pairs = ((w1_hbm, w1_v), (w2_hbm, w2_v), (w3_hbm, w3_v), (w4_hbm, w4_v), (wo_hbm, wo_v))

    def w_start(j, part=0, parts=1, priority=0):
        src, dst = w_pairs[j]
        tiles = dst.shape[0]
        for n in range(part * tiles // parts, (part + 1) * tiles // parts):
            pltpu.make_async_copy(src.at[:, pl.ds(n * _LANES, _LANES)], dst.at[n],
                                  sem_w.at[j]).start(priority=priority)

    def w_wait(j):
        dst = w_pairs[j][1]
        pltpu.make_async_copy(dst, dst, sem_w.at[j]).wait()

    def stage_copy(i, j):
        src = (wq_hbm, wk_hbm, wv_hbm)[j]
        rows = pl.ds(pl.multiple_of(i * (db * H), db * H), db * H)
        slot = (i % 2) * 3 + j
        return pltpu.make_async_copy(src.at[rows], stage_v.at[slot], sem_st.at[slot])

    def stage_start(i):
        for j in range(3):
            stage_copy(i, j).start()

    def out_copy(s):
        rows = pl.ds(pl.multiple_of(s * seg, seg), seg)
        return pltpu.make_async_copy(x_v.at[rows], out_hbm.at[rows], sem_io.at[0])

    mem0_copy = pltpu.make_async_copy(mem0_hbm, mem0_v, sem_io.at[1])

    def paced(i, steps, jobs):
        per = -(-len(jobs) // steps)
        for k in range(steps):
            mine = jobs[k * per:(k + 1) * per]
            if mine:
                @pl.when(i == k)
                def _(mine=mine):
                    for job in mine:
                        job()

    part = functools.partial
    jobs_p = [part(w_start, 1, 0, 1, 1)] + [part(w_start, 2, k, 4, 1) for k in range(3)]
    jobs_q = ([part(w_start, 2, 3, 4)] + [part(w_start, 3, k, 4) for k in range(4)]
              + [part(stage_start, 0)] + [part(w_start, 4, k, 2) for k in range(2)])

    x_copy(0).start()
    w_start(0)
    x_copy(1).start()
    x_copy(2).start()
    hb_v[0:_PAD, :] = jnp.zeros((_PAD, D), _F32)
    hb_v[_PAD + S:, :] = jnp.zeros((_PAD, D), _F32)

    def norms(dst_v, src0, dst0, rows):
        xn = _layernorm(x_v[pl.ds(src0, rows), :].astype(_F32))
        xn_v[pl.ds(src0, rows), :] = xn
        ln = _layernorm(xn)
        dst_v.bitcast(_BF16)[pl.ds(dst0, rows), :] = ln.astype(_BF16)
        return ln

    def next_block(fn, blk, rows, first, last, zero):
        nxt = jnp.minimum(blk + 1, n_blk - 1) * _TB
        groups = _TB // rows
        return {first + g * (last - first) // (groups - 1):
                _token(fn(pl.multiple_of(nxt + g * rows, rows), g * rows, rows), zero)
                for g in range(groups)}

    x_copy(0).wait()
    norms(la_v, 0, 0, _TB)
    mem0_copy.start()
    w_wait(0)

    def phase_p(i, carry):
        paced(i, n_blk // 2, jobs_p)
        for k in (3, 4):
            @pl.when(2 * i + k < n_blk)
            def _(k=k):
                x_copy(2 * i + k).start()

        x_copy(2 * i + 1).wait()

        @pl.when(2 * i + 2 < n_blk)
        def _():
            x_copy(2 * i + 2).wait()

        zero = pltpu.bitcast(hb_v[0:8, 0:_LANES], _U32)
        for k, (cur_v, nxt_v) in enumerate(((la_v, lb_v), (lb_v, la_v))):
            blk = 2 * i + k
            r0 = pl.multiple_of(blk * _TB, _TB)
            after = next_block(functools.partial(norms, nxt_v), blk, 64, 5, 15, zero)
            pre = _matmul(cur_v.bitcast(_BF16)[...], w1_v, after)
            hb_v[pl.ds(r0 + _PAD, _TB), :] = _gelu(pre)
        return carry

    jax.lax.fori_loop(0, n_blk // 2, phase_p, 0)

    w_wait(1)

    def phase_q(i, carry):
        paced(i, n_blk, jobs_q)
        r0 = pl.multiple_of(i * _TB, _TB)
        parts = []
        for q, shift in enumerate((-1, 1, -2, 2)):
            win = hb_v[pl.ds(r0, _TB + 2 * _PAD), q * c:(q + 1) * c]
            parts.append(win[_PAD + shift:_PAD + shift + _TB])
        x1_v[pl.ds(r0, _TB), :] = (xn_v[pl.ds(r0, _TB), :]
                                   + _matmul(jnp.concatenate(parts, axis=1), w2_v))
        return carry

    jax.lax.fori_loop(0, n_blk, phase_q, 0)

    def norm3(src0, dst0, rows):
        ln = _layernorm(x1_v[pl.ds(src0, rows), :])
        la_v.bitcast(_BF16)[pl.ds(dst0, rows), :] = ln.astype(_BF16)
        return ln

    norm3(0, 0, _TB)
    w_wait(2)
    w_wait(3)
    stage_u = stage_v.bitcast(_U32)

    def phase_r(i, carry):
        @pl.when(i + 1 < n_blk)
        def _():
            stage_start(i + 1)

        for j in range(3):
            stage_copy(i, j).wait()

        zero = pltpu.bitcast(hb_v[0:8, 0:_LANES], _U32)

        def relayout(j, g, t, odd, z):
            keep, sh = z | _U32(0xFFFF0000 if odd else 0xFFFF), z | _U32(16)
            j0 = pl.multiple_of(i * (db // 2) + g * 8, 8)
            w = stage_u[(i % 2) * 3 + j, g * 8 * H:(g + 1) * 8 * H, :].reshape(8, H, _LANES)
            a = w[:, 8 * t:8 * t + 8, :]
            b = w[:, H // 2 + 8 * t:H // 2 + 8 * t + 8, :]
            word = ((a >> sh) | (b & keep)) if odd else ((a & keep) | (b << sh))
            word = jnp.transpose(word, (1, 0, 2))
            for r in range(8):
                wqkv_v[(2 * (8 * t + r) + odd) * 3 + j, pl.ds(j0, 8), :] = word[r]

        pieces = [(j, g, t, odd) for j in range(3) for g in range(db // 16)
                  for t in range(H // 16) for odd in range(2)]

        r0 = pl.multiple_of(i * _TB, _TB)
        pre = _matmul(la_v.bitcast(_BF16)[...], w3_v)
        for z in _anchors(pre, len(pieces), zero):
            relayout(*pieces.pop(), z)
        after = next_block(norm3, i, 32, 4, 36, zero)
        y = x1_v[pl.ds(r0, _TB), :] + _matmul(_gelu(pre).astype(_BF16), w4_v, after)
        hb_v[pl.ds(r0 + _PAD, _TB), :] = y * jax.nn.sigmoid(y)
        return carry

    jax.lax.fori_loop(0, n_blk, phase_r, 0)

    w_wait(4)
    wo_u = wo_v.bitcast(_U32)
    mem0_copy.wait()
    h_v[0:M, :] = mem0_v[...].astype(_F32)
    h_early = H - H // 4

    def proj(h, j):
        return _dot(h_v[...], pltpu.bitcast(wqkv_v[h * 3 + j], _BF16))

    def first_proj():
        kh = D // 2
        for j in range(3):
            acc_v[:, j * _LANES:(j + 1) * _LANES] = _dot(
                h_v[:, :kh], pltpu.bitcast(wqkv_v[j, :kh // 2, :], _BF16))
        return tuple(
            acc_v[:, j * _LANES:(j + 1) * _LANES]
            + _dot(h_v[:, kh:], pltpu.bitcast(wqkv_v[j, kh // 2:, :], _BF16)) for j in range(3))

    def out_proj(n, h0, h1):
        w = wo_u[n, h0 * (_LANES // 2):h1 * (_LANES // 2), :]
        return _dot(o_v[:, h0 * _LANES:h1 * _LANES], pltpu.bitcast(w, _BF16))

    def step(s, carry):
        r0 = pl.multiple_of(s * seg, seg)
        h_v[M:L, :] = xn_v[pl.ds(r0, seg), :]
        qi = jax.lax.broadcasted_iota(jnp.int32, (L, L), 0)
        ki = jax.lax.broadcasted_iota(jnp.int32, (L, L), 1)
        mask = (qi < M) | (qi >= ki)
        qkv, prob = {}, {}

        def scores(h):
            q, k, _ = qkv[h]
            sc = jax.lax.dot_general(q, k, (((1,), (1,)), ((), ())),
                                     preferred_element_type=_F32)
            sc = jnp.where(mask, sc * scale, -1000000000.0)
            p = jnp.exp(sc - jnp.max(sc, axis=-1, keepdims=True))
            prob[h] = p / jnp.sum(p, axis=-1, keepdims=True)

        def values(h):
            o_v[:, h * _LANES:(h + 1) * _LANES] = _dot(prob.pop(h), qkv.pop(h)[2])

        for t in range(H + n_col):
            if t == 0:
                qkv[t] = first_proj()
            elif t < H:
                qkv[t] = (proj(t, 0), proj(t, 1), proj(t, 2))
            else:
                n = t - H
                acc_v[:, n * _LANES:(n + 1) * _LANES] = out_proj(n, 0, h_early)
            if 0 <= t - _LAG_S < H:
                scores(t - _LAG_S)
            if 0 <= t - _LAG_V < H:
                values(t - _LAG_V)

        for n in range(n_col):
            cols = slice(n * _LANES, (n + 1) * _LANES)
            o = acc_v[:, cols] + out_proj(n, h_early, H)
            h_v[0:M, cols] = o[0:M]
            res = (x_v[pl.ds(r0, seg), cols].astype(_F32)
                   + o[M:L] * hb_v[pl.ds(r0 + _PAD, seg), cols])
            x_v[pl.ds(r0, seg), cols] = res.astype(x_v.dtype)
        out_copy(s).start()
        return carry

    jax.lax.fori_loop(0, n_seg, step, 0, unroll=2)
    pltpu.make_async_copy(x_v, out_hbm, sem_io.at[0]).wait()


@functools.partial(jax.jit, static_argnames=("A_seg_len",))
def pallas_recurrent_scan__memory_aug_recurrent_mem_tr__mixer_s_mlp__prompt_kernel(
    A_x, A_mem0, A_Wq, A_Wk, A_Wv, A_Wo, A_seg_len, B_x, B_w1, B_w2, B_w3, B_w4,
):
    del B_x
    B, S, D = A_x.shape
    M = A_mem0.shape[1]
    _, H, Dh = A_Wq.shape
    F = B_w3.shape[1]
    seg = int(A_seg_len)
    n_blk = S // _TB
    n_col = D // _LANES
    assert B == 1 and Dh == _LANES and S % (2 * _TB) == 0 and n_blk >= 4
    assert S % (2 * seg) == 0 and seg % 16 == 0 and M % 8 == 0 and M + seg <= _LANES
    assert H % 16 == 0 and D % (16 * n_blk) == 0 and _LAG_V <= min(n_col, H // 4)

    out = pl.pallas_call(
        functools.partial(_kernel, seg=seg, n_heads=H),
        out_shape=jax.ShapeDtypeStruct((S, D), A_x.dtype),
        in_specs=[pl.BlockSpec(memory_space=pl.ANY)] * 10,
        out_specs=pl.BlockSpec(memory_space=pl.ANY),
        scratch_shapes=[
            pltpu.VMEM((S, D), _BF16),
            pltpu.VMEM((S, D), _F32),
            pltpu.VMEM((S + 2 * _PAD, D), _F32),
            pltpu.VMEM((S, D), _F32),
            pltpu.VMEM((_TB // 2, D), _U32),
            pltpu.VMEM((_TB // 2, D), _U32),
            pltpu.VMEM((3 * H, D // 2, Dh), _U32),
            pltpu.VMEM((n_col, H * Dh, _LANES), _BF16),
            pltpu.VMEM((n_col, D, _LANES), _BF16),
            pltpu.VMEM((n_col, D, _LANES), _BF16),
            pltpu.VMEM((F // _LANES, D, _LANES), _BF16),
            pltpu.VMEM((n_col, F, _LANES), _BF16),
            pltpu.VMEM((6, (D // n_blk) * H, Dh), _BF16),
            pltpu.VMEM((M + seg, D), _F32),
            pltpu.VMEM((M + seg, H * Dh), _F32),
            pltpu.VMEM((M + seg, D), _F32),
            pltpu.VMEM((M, D), _BF16),
            pltpu.SemaphoreType.DMA((n_blk,)),
            pltpu.SemaphoreType.DMA((5,)),
            pltpu.SemaphoreType.DMA((6,)),
            pltpu.SemaphoreType.DMA((2,)),
        ],
        compiler_params=pltpu.CompilerParams(vmem_limit_bytes=120 * 1024 * 1024),
    )(
        A_x.reshape(S, D), A_mem0.reshape(M, D),
        A_Wq.reshape(D * H, Dh), A_Wk.reshape(D * H, Dh), A_Wv.reshape(D * H, Dh),
        A_Wo.reshape(H * Dh, D), B_w1, B_w2, B_w3, B_w4,
    )
    return out.reshape(B, S, D)
```
